```python
import os as _os
_os.environ.setdefault("JAX_PLATFORMS", "cpu")
import jax
import jax.numpy as jnp

def _softmax(x, axis=-1):
    return jax.nn.softmax(x, axis=axis)
def _gelu(x):
    return jax.nn.gelu(x, approximate=True)
def _silu(x):
    return jax.nn.silu(x)
def _sigmoid(x):
    return jax.nn.sigmoid(x)
def _layernorm(x, axis=-1, eps=1e-5):
    m = jnp.mean(x, axis=axis, keepdims=True)
    v = jnp.var(x, axis=axis, keepdims=True)
    return (x - m) / jnp.sqrt(v + eps)
def _scatter_add(tgt, idx, src, axis=0):
    return tgt.at[idx].add(src)
def _segment_sum(src, seg, n):
    return jax.ops.segment_sum(src, seg, n)
class _Rng:
    def __init__(self, key):
        self._k = key
    def _next(self):
        self._k, sub = jax.random.split(self._k)
        return sub
    def normal(self, shape):
        return jax.random.normal(self._next(), shape, dtype=jnp.bfloat16)
    def randint(self, lo, hi, shape):
        return jax.random.randint(self._next(), shape, lo, hi, dtype=jnp.int32)
    def uniform(self, shape, lo=0.0, hi=1.0):
        return jax.random.uniform(self._next(), shape, jnp.bfloat16, lo, hi)
    def permutation(self, n):
        return jax.random.permutation(self._next(), n)


kernel_name = 'standalone__gqa_block_cached__near_ridge'

def setup_inputs():
    _rng = _Rng(jax.random.key(int.from_bytes(__import__("os").urandom(4), "little")))
    _w = (lambda a: (lambda t: t.astype(jnp.bfloat16) if jnp.issubdtype(t.dtype, jnp.floating) else t)(jnp.asarray(a)))
    B, Sq, D = 8, 144, 448
    Hq, Hkv, Sk, Dh = 16, 8, 2048, 256
    assert Hq % Hkv == 0, (Hq, Hkv)
    return {
        "x": _w((lambda *s: _rng.normal(s) * 0.8)(B, Sq, D)),
        "k_cache": _w((lambda *s: _rng.normal(s) * 0.8)(B, Hkv, Sk, Dh)),
        "v_cache": _w((lambda *s: _rng.normal(s) * 0.05)(B, Hkv, Sk, Dh)),
        "wq": _w((lambda *s: _rng.normal(s) * 0.8)(D, Hq * Dh) * (D ** -0.5)),
        "wo": _w((lambda *s: _rng.normal(s) * 0.05)(Hq * Dh, D) * ((Hq * Dh) ** -0.5)),
    }

def reference(x, k_cache, v_cache, wq, wo):
    B, Sq, D = x.shape
    Hq, Dh = 16, 256
    Hkv = k_cache.shape[1]
    rep = Hq // Hkv
    q = (lambda x, *d: x.transpose(*d))((x @ wq).reshape(B, Sq, Hq, Dh), 0, 2, 1, 3)
    k = jnp.repeat(k_cache, rep, axis=1)
    v = jnp.repeat(v_cache, rep, axis=1)
    scores = jnp.einsum("bhqd,bhkd->bhqk", q, k) * (Dh ** -0.5)
    p = _softmax(scores, axis=-1)
    o = jnp.einsum("bhqk,bhkd->bhqd", p, v)
    return (lambda x, *d: x.transpose(*d))(o, 0, 2, 1, 3).reshape(B, Sq, Hq * Dh) @ wo
```

```python
import functools
import jax
import jax.numpy as jnp
from jax import lax
import jax.experimental.pallas as pl
import jax.experimental.pallas.tpu as pltpu

LOG2E = 1.4426950408889634

def _make(P=4, KC=512, vmem=110, NBUF=3, checks=False, dmode='T', DG=1, recip='newton'):
    def _recip(l):
        if recip == 'exact':
            return pl.reciprocal(l, approx=False)
        r = pl.reciprocal(l, approx=True)
        return r * (2.0 - l * r)

    def fn(x, k_cache, v_cache, wq, wo):
        B, Sq, D = x.shape
        _, Hkv, Sk, Dh = k_cache.shape
        Hq = wq.shape[1] // Dh
        rep = Hq // Hkv
        M = rep * Sq
        W = rep * Dh
        scale = Dh ** -0.5 * LOG2E
        woT = wo.T
        NP = B * Hkv
        NS = NP // P
        SPH = B // P
        NT = (((1,), (1,)), ((), ()))
        NC = Sk // KC
        f32, bf16 = jnp.float32, jnp.bfloat16

        def kernel(x_hbm, k_hbm, v_hbm, wq_hbm, wo_hbm, out_hbm,
                   x_v, wq_v, wo_v, kbuf, vbuf, q_all, ou_all, l_all, acc_scr, accT_scr, out_v, s_scr, m_scr,
                   ksem, vsem, wsem, osem):
            def blk(t):
                return t // SPH, (t % SPH) * P
            def kcopy(t):
                h, b0 = blk(t)
                slot = t % NBUF
                return pltpu.make_async_copy(k_hbm.at[pl.ds(b0, P), h], kbuf.at[slot], ksem.at[slot])
            def vcopy(t):
                h, b0 = blk(t)
                slot = t % NBUF
                return pltpu.make_async_copy(v_hbm.at[pl.ds(b0, P), h], vbuf.at[slot], vsem.at[slot])
            xcopy = pltpu.make_async_copy(x_hbm, x_v, wsem.at[0])
            def wqcopy(h):
                return pltpu.make_async_copy(wq_hbm.at[:, pl.ds(h * W, W)], wq_v.at[h], wsem.at[2 + h])
            def wocopy(h):
                return pltpu.make_async_copy(wo_hbm.at[:, pl.ds(h * W, W)], wo_v.at[h], wsem.at[1])

            xcopy.start()
            for h in range(Hkv):
                wqcopy(h).start()
            if dmode == 'T':
                accT_scr[...] = jnp.zeros_like(accT_scr)
            else:
                acc_scr[...] = jnp.zeros_like(acc_scr)
            xcopy.wait()
            kcopy(0).start()
            kcopy(1).start()
            vcopy(0).start()
            for t in range(2, NBUF):
                kcopy(t).start()
                vcopy(t - 1).start()

            def qbody(h, c):
                wqcopy(h).wait()
                xx = x_v[...].reshape(B * Sq, D)
                q = jnp.dot(xx, wq_v[h], preferred_element_type=f32)
                q = (q * scale).astype(bf16)
                for bb in range(B):
                    for r in range(rep):
                        q_all[h, bb, r * Sq:(r + 1) * Sq, :] = q[bb * Sq:(bb + 1) * Sq, r * Dh:(r + 1) * Dh]
                return c
            lax.fori_loop(0, Hkv, qbody, 0)

            def sub(i, t, do_qk, do_pv, split_last):
                if do_pv:
                    hp, bp0 = blk(t - 1)
                    bp = bp0 + i
                    vslot = (t - 1) % NBUF
                if do_qk:
                    h, b0 = blk(t)
                    kslot = t % NBUF
                mrun = None
                o = None
                l = None
                for j in range(NC):
                    last = j == NC - 1
                    ks = slice(j * KC, (j + 1) * KC)
                    if do_pv:
                        m = m_scr[i]
                        pj = jnp.exp2(s_scr[i, :, ks] - jnp.concatenate([m] * (KC // 128), axis=1))
                        lj = None
                        for c in range(KC // 128):
                            pc = pj[:, c * 128:(c + 1) * 128]
                            lj = pc if lj is None else lj + pc
                        l = lj if l is None else l + lj
                        pb = pj.astype(bf16)
                        if last:
                            l_all[hp, bp] = l
                        if last and split_last:
                            oa = jnp.dot(pb, vbuf[vslot, i, ks, 0:128], preferred_element_type=f32)
                            ou_all[hp, bp, :, 0:128] = oa + o[:, 0:128]
                        else:
                            oj = jnp.dot(pb, vbuf[vslot, i, ks, :], preferred_element_type=f32)
                            o = oj if o is None else oj + o
                            if last:
                                ou_all[hp, bp] = o
                    if do_qk:
                        s = lax.dot_general(q_all[h, b0 + i], kbuf[kslot, i, ks, :], NT, preferred_element_type=f32)
                        s_scr[i, :, ks] = s
                        for c in range(KC // 128):
                            sc = s[:, c * 128:(c + 1) * 128]
                            mrun = sc if mrun is None else jnp.maximum(mrun, sc)
                        if last:
                            m_scr[i] = jnp.broadcast_to(jnp.max(mrun, axis=-1, keepdims=True), (M, 128))
                    if do_pv and last and split_last:
                        ob = jnp.dot(pb, vbuf[vslot, i, ks, 128:256], preferred_element_type=f32)
                        ou_all[hp, bp, :, 128:256] = ob + o[:, 128:256]

            kcopy(0).wait()
            def a2(i, c):
                sub(i, 0, True, False, False)
                return c
            lax.fori_loop(0, P, a2, 0)

            def body(t, c):
                kcopy(t).wait()
                vcopy(t - 1).wait()
                @pl.when(t + NBUF - 1 < NS)
                def _():
                    kcopy(t + NBUF - 1).start()
                @pl.when(t + NBUF - 2 < NS)
                def _():
                    vcopy(t + NBUF - 2).start()
                @pl.when(t <= Hkv)
                def _():
                    wocopy(t - 1).start()
                for i in range(P):
                    sub(i, t, True, True, i == P - 1)
                return c
            lax.fori_loop(1, NS, body, 0)

            vcopy(NS - 1).wait()
            for h in range(Hkv):
                wocopy(h).wait()
            def cbody(i, c):
                sub(i, NS, False, True, False)
                return c
            lax.fori_loop(0, P, cbody, 0)

            def normed(h, b):
                l = jnp.sum(l_all[h, b], axis=-1, keepdims=True)
                o = ou_all[h, b] * _recip(l)
                return jnp.concatenate([o[r * Sq:(r + 1) * Sq] for r in range(rep)], axis=1).astype(bf16)
            def dbody(h, c):
                if dmode == 'batch':
                    for g in range(B // DG):
                        on = jnp.concatenate([normed(h, g * DG + k) for k in range(DG)], axis=0)
                        y = lax.dot_general(on, wo_v[h], NT, preferred_element_type=f32)
                        acc_scr[g * DG * Sq:(g + 1) * DG * Sq, :] += y
                else:
                    on = jnp.concatenate([normed(h, b) for b in range(B)], axis=0)
                    y = lax.dot_general(wo_v[h], on, NT, preferred_element_type=f32)
                    accT_scr[...] += y
                return c
            lax.fori_loop(0, Hkv, dbody, 0)
            if dmode == 'T':
                out_v[...] = accT_scr[...].T.astype(bf16).reshape(B, Sq, D)
            else:
                out_v[...] = acc_scr[...].astype(bf16).reshape(B, Sq, D)
            oc = pltpu.make_async_copy(out_v, out_hbm, osem)
            oc.start()
            oc.wait()

        out = pl.pallas_call(
            kernel,
            in_specs=[pl.BlockSpec(memory_space=pl.ANY)] * 5,
            out_specs=pl.BlockSpec(memory_space=pl.ANY),
            out_shape=jax.ShapeDtypeStruct((B, Sq, D), x.dtype),
            scratch_shapes=[
                pltpu.VMEM((B, Sq, D), bf16),
                pltpu.VMEM((Hkv, D, W), bf16),
                pltpu.VMEM((Hkv, D, W), bf16),
                pltpu.VMEM((NBUF, P, Sk, Dh), bf16),
                pltpu.VMEM((NBUF, P, Sk, Dh), bf16),
                pltpu.VMEM((Hkv, B, M, Dh), bf16),
                pltpu.VMEM((Hkv, B, M, Dh), f32),
                pltpu.VMEM((Hkv, B, M, 128), f32),
                pltpu.VMEM((B * Sq, D), f32),
                pltpu.VMEM((D, B * Sq), f32),
                pltpu.VMEM((B, Sq, D), bf16),
                pltpu.VMEM((P, M, Sk), f32),
                pltpu.VMEM((P, M, 128), f32),
                pltpu.SemaphoreType.DMA((NBUF,)),
                pltpu.SemaphoreType.DMA((NBUF,)),
                pltpu.SemaphoreType.DMA((2 + Hkv,)),
                pltpu.SemaphoreType.DMA,
            ],
            compiler_params=pltpu.CompilerParams(
                vmem_limit_bytes=vmem * 1024 * 1024,
                disable_bounds_checks=not checks,
                disable_semaphore_checks=not checks,
            ),
        )(x, k_cache, v_cache, wq, woT)
        return out
    return fn


@jax.jit
def pallas_standalone__gqa_block_cached__near_ridge_kernel(x, k_cache, v_cache, wq, wo):
    return _make()(x, k_cache, v_cache, wq, wo)
```

```python
import functools
import jax
import jax.numpy as jnp
from jax import lax
import jax.experimental.pallas as pl
import jax.experimental.pallas.tpu as pltpu

LOG2E = 1.4426950408889634

def _make(KC=512, vmem=100, checks=False, xsplit=2, out_groups=(1, 2, 3, 4, 5, 6, 7, 8, 9), dma_at=1, eager=False, bar=7, nnorm=1, CU=2, amid=3, lag=2, pad=0):
    P = 4
    NBUF = 3
    def _recip(l):
        r = pl.reciprocal(l, approx=True)
        return r * (2.0 - l * r)

    def fn(x, k_cache, v_cache, wq, wo):
        B, Sq, D = x.shape
        _, Hkv, Sk, Dh = k_cache.shape
        Hq = wq.shape[1] // Dh
        rep = Hq // Hkv
        M = rep * Sq
        W = rep * Dh
        R = B * Sq
        TPH = W // 128
        TPQ = Dh // 128
        NTL = Hq * Dh // 128
        G = (NTL - TPH) // P
        assert G * P == NTL - TPH
        scale = Dh ** -0.5 * LOG2E
        x2 = x.reshape(R, D)
        woT = wo.T
        NP = B * Hkv
        NS = NP // P
        SPH = B // P
        assert SPH == 2
        NT = (((1,), (1,)), ((), ()))
        NC = Sk // KC
        f32, bf16 = jnp.float32, jnp.bfloat16
        XR = xsplit * Sq

        def kernel(x_hbm, k_hbm, v_hbm, wq_hbm, wo_hbm, out_hbm,
                   x_v, wq0_v, wqr_v, wor_v, wo7_v, kbuf, vbuf, q0, q_all, ou_all, l_all, ou7, l7,
                   accT, out_v, s_scr, m_scr, on_scr, rt_scr, acc_n, bsem,
                   ksem, vsem, k0sem, wqsem, wsem, osem):
            def blk(t):
                if isinstance(t, int):
                    return t // SPH, (t % SPH) * P
                return lax.shift_right_logical(t, 1), (t & 1) * P
            def kcopy(t, slot):
                h, b0 = blk(t)
                return pltpu.make_async_copy(k_hbm.at[pl.ds(b0, P), h], kbuf.at[slot], ksem.at[slot])
            def vcopy(t, slot):
                h, b0 = blk(t)
                return pltpu.make_async_copy(v_hbm.at[pl.ds(b0, P), h], vbuf.at[slot], vsem.at[slot])
            def k0copy(i):
                return pltpu.make_async_copy(k_hbm.at[i, 0], kbuf.at[0, i], k0sem.at[i])
            xa = pltpu.make_async_copy(x_hbm.at[pl.ds(0, XR)], x_v.at[pl.ds(0, XR)], wsem.at[0])
            xb = pltpu.make_async_copy(x_hbm.at[pl.ds(XR, R - XR)], x_v.at[pl.ds(XR, R - XR)], wsem.at[1])
            wq0c = pltpu.make_async_copy(wq_hbm.at[:, pl.ds(0, W)], wq0_v, wsem.at[2])
            def wqrc(i):
                return pltpu.make_async_copy(wq_hbm.at[:, pl.ds(W + i * G * 128, G * 128)], wqr_v.at[i], wqsem.at[i])
            worc = [pltpu.make_async_copy(wo_hbm.at[:, pl.ds(i * G * 128, G * 128)], wor_v.at[i], wsem.at[3]) for i in range(P)]
            wo7c = pltpu.make_async_copy(wo_hbm.at[:, pl.ds(P * G * 128, W)], wo7_v, wsem.at[3])

            xa.start()
            wq0c.start()
            xb.start()
            accT[...] = jnp.zeros_like(accT)

            HR = P * Sq
            def qproj(w, tile0, r0, r1, first=False):
                q = jnp.dot(x_v[r0:r1, :], w, preferred_element_type=f32)
                q = (q * scale).astype(bf16)
                for k in range(w.shape[1] // 128):
                    qk_ = q[:, k * 128:(k + 1) * 128]
                    if first:
                        if r0 < HR:
                            q0[k, r0:min(r1, HR), :] = qk_[0:min(r1, HR) - r0]
                        if r1 > HR:
                            q_all[k, max(r0, HR):r1, :] = qk_[max(r0, HR) - r0:]
                    else:
                        q_all[tile0 + k, r0:r1, :] = qk_

            xa.wait()
            wq0c.wait()
            k0copy(0).start()
            wqrc(0).start()
            qproj(wq0_v[...], 0, 0, XR, True)
            xb.wait()
            k0copy(1).start()
            wqrc(1).start()
            if eager:
                for i in range(2, P):
                    k0copy(i).start()
                    wqrc(i).start()
                kcopy(1, 1).start()
                vcopy(0, 0).start()
                kcopy(2, 2).start()
                vcopy(1, 1).start()
            qproj(wq0_v[...], 0, XR, R, True)

            def load_q(h, b):
                qsrc = q0 if isinstance(h, int) else q_all
                row = b * Sq
                if not isinstance(row, int):
                    row = pl.multiple_of(row, 16)
                rows = []
                for r in range(rep):
                    rows.append(jnp.concatenate(
                        [qsrc[h * TPH + r * TPQ + c, pl.ds(row, Sq), :] for c in range(TPQ)], axis=1))
                return jnp.concatenate(rows, axis=0)

            def sub(i, qk, pv, split_last):
                mrun = None
                o = None
                l = None
                for j in range(NC):
                    last = j == NC - 1
                    ks = slice(j * KC, (j + 1) * KC)
                    if pv is not None:
                        store_o, store_l, vslot = pv
                        m = m_scr[i]
                        pj = jnp.exp2(s_scr[i, :, ks] - jnp.concatenate([m] * (KC // 128), axis=1))
                        lj = None
                        for c in range(KC // 128):
                            pc = pj[:, c * 128:(c + 1) * 128]
                            lj = pc if lj is None else lj + pc
                        l = lj if l is None else l + lj
                        pb = pj.astype(bf16)
                        if last:
                            store_l(l)
                        if last and split_last:
                            oa = jnp.dot(pb, vbuf[vslot, i, ks, 0:128], preferred_element_type=f32)
                            store_o(0, oa + o[:, 0:128])
                        else:
                            oj = jnp.dot(pb, vbuf[vslot, i, ks, :], preferred_element_type=f32)
                            o = oj if o is None else oj + o
                            if last:
                                for c in range(TPQ):
                                    store_o(c, o[:, c * 128:(c + 1) * 128])
                    if qk is not None:
                        h, b, kslot = qk
                        s = lax.dot_general(load_q(h, b), kbuf[kslot, i, ks, :], NT, preferred_element_type=f32)
                        s_scr[i, :, ks] = s
                        for c in range(KC // 128):
                            sc = s[:, c * 128:(c + 1) * 128]
                            mrun = sc if mrun is None else jnp.maximum(mrun, sc)
                        if last:
                            m_scr[i] = jnp.broadcast_to(jnp.max(mrun, axis=-1, keepdims=True), (M, 128))
                    if pv is not None and last and split_last:
                        ob = jnp.dot(pb, vbuf[vslot, i, ks, 128:256], preferred_element_type=f32)
                        store_o(1, ob + o[:, 128:256])

            def abody(i, c):
                k0copy(i).wait()
                wqrc(i).wait()
                if amid:
                    qproj(wqr_v[i, :, 0:amid * 128], TPH + i * G, 0, R)
                @pl.when(i + 2 < P)
                def _():
                    k0copy(i + 2).start()
                    wqrc(i + 2).start()
                @pl.when(i == 0)
                def _():
                    kcopy(1, 1).start()
                @pl.when(i == 1)
                def _():
                    vcopy(0, 0).start()
                @pl.when(i == 2)
                def _():
                    kcopy(2, 2).start()
                @pl.when(i == 3)
                def _():
                    vcopy(1, 1).start()
                sub(i, (0, i, 0), None, False)
                qproj(wqr_v[i, :, amid * 128:], TPH + i * G + amid, 0, R)
                return c
            lax.fori_loop(0, P, abody, 0)

            def body(t, slots):
                sm1, s0, sp1 = slots
                kcopy(t, s0).wait()
                vcopy(t - 1, sm1).wait()
                h, b0 = blk(t)
                hp, bp0 = blk(t - 1)
                def issue():
                    @pl.when(t + 2 < NS)
                    def _():
                        kcopy(t + 2, sm1).start()
                    @pl.when(t + 1 < NS)
                    def _():
                        vcopy(t + 1, sp1).start()
                    @pl.when(t == 1)
                    def _():
                        for cc in worc:
                            cc.start()
                        wo7c.start()
                for i in range(P):
                    if i == dma_at:
                        issue()
                    row = pl.multiple_of((bp0 + i) * Sq, 16)
                    def store_o(c, val, row=row):
                        for r in range(rep):
                            ou_all[hp * TPH + r * TPQ + c, pl.ds(row, Sq), :] = val[r * Sq:(r + 1) * Sq]
                    def store_l(val, row=row):
                        for r in range(rep):
                            l_all[hp * rep + r, pl.ds(row, Sq), :] = val[r * Sq:(r + 1) * Sq]
                    sub(i, (h, b0 + i, s0), (store_o, store_l, sm1), i == P - 1)
                return (s0, sp1, sm1)
            fin = lax.fori_loop(1, NS, body, (jnp.int32(0), jnp.int32(1), jnp.int32(2)))
            zero = fin[(NBUF - (NS - 1) % NBUF) % NBUF]

            vlast = (NS - 1) % NBUF
            vcopy(NS - 1, vlast).wait()
            for cc in worc:
                cc.wait()
            wo7c.wait()
            def cbody(ii, c):
                for u in range(CU):
                    i = ii * CU + u
                    row = pl.multiple_of(i * Sq, 16)
                    def store_o(cc, val, row=row):
                        for r in range(rep):
                            ou7[r * TPQ + cc, pl.ds(row, Sq), :] = val[r * Sq:(r + 1) * Sq]
                    def store_l(val, row=row):
                        for r in range(rep):
                            l7[r, pl.ds(row, Sq), :] = val[r * Sq:(r + 1) * Sq]
                    sub(i, None, (store_o, store_l, vlast), False)
                tiles = []
                if CU % 2 == 0:
                    for k2 in range(CU * G // 2):
                        kq = ii * (CU * G // 2) + k2
                        rc = _recip(jnp.sum(l_all[kq, 0:R, :], axis=-1, keepdims=True))
                        for cc in range(TPQ):
                            tiles.append(ou_all[kq * TPQ + cc, 0:R, :] * rc)
                else:
                    for k in range(CU * G):
                        kt = ii * CU * G + k
                        l = jnp.sum(l_all[lax.shift_right_logical(kt, 1)], axis=-1, keepdims=True)
                        tiles.append(ou_all[kt] * _recip(l))
                on = jnp.concatenate(tiles, axis=1).astype(bf16)
                w = jnp.concatenate([wor_v[ii * CU + u] for u in range(CU)], axis=1)
                accT[...] += lax.dot_general(w, on, NT, preferred_element_type=f32)
                return c
            lax.fori_loop(0, P // CU, cbody, 0)

            def rows_of(big, small, idx_big, idx_small, r0, r1):
                parts = []
                if r0 < HR:
                    parts.append(big[idx_big, r0:min(r1, HR), :])
                if r1 > HR:
                    parts.append(small[idx_small, max(r0, HR) - HR:r1 - HR, :])
                return parts[0] if len(parts) == 1 else jnp.concatenate(parts, axis=0)
            ocs = []
            prev = 0
            def emit(n, resT):
                nonlocal prev
                r0, r1 = n * 128, (n + 1) * 128
                out_v[pl.ds(pl.multiple_of(r0 + zero, 128), 128), :] = resT
                if n + 1 in out_groups:
                    oc = pltpu.make_async_copy(out_v.at[pl.ds(prev, r1 - prev)], out_hbm.at[pl.ds(prev, r1 - prev)],
                                               osem.at[len(ocs)])
                    oc.start()
                    ocs.append(oc)
                    prev = r1
            def normed7(n):
                r0, r1 = n * 128, (n + 1) * 128
                tiles = []
                for r in range(rep):
                    l = jnp.sum(rows_of(l_all, l7, (Hkv - 1) * rep + r, r, r0, r1), axis=-1, keepdims=True)
                    rc = _recip(l)
                    for cc in range(TPQ):
                        tiles.append(rows_of(ou_all, ou7, (Hkv - 1) * TPH + r * TPQ + cc, r * TPQ + cc, r0, r1) * rc)
                return jnp.concatenate(tiles, axis=1).astype(bf16)
            NO = R // 128
            for n in range(NO - nnorm, NO):
                acc_n[n - NO + nnorm] = accT[:, n * 128:(n + 1) * 128].T
            res = {}
            for n in range(NO + lag):
                if n >= lag:
                    emit(n - lag, res.pop(n - lag))
                if n >= NO:
                    continue
                r0, r1 = n * 128, (n + 1) * 128
                on = normed7(n)
                if n >= lag:
                    rows = pl.ds(pl.multiple_of(r0 + zero, 128), 128)
                    out_v[rows, 0:128] = on[:, 0:128]
                    on = jnp.concatenate([out_v[rows, 0:128], on[:, 128:]], axis=1)
                if n >= NO - nnorm:
                    res[n] = (lax.dot_general(on, wo7_v[...], NT, preferred_element_type=f32) + acc_n[n - NO + nnorm]).astype(bf16)
                else:
                    res[n] = (lax.dot_general(wo7_v[...], on, NT, preferred_element_type=f32) + accT[:, r0:r1]).astype(bf16).T
            for oc in ocs:
                oc.wait()

        out = pl.pallas_call(
            kernel,
            in_specs=[pl.BlockSpec(memory_space=pl.ANY)] * 5,
            out_specs=pl.BlockSpec(memory_space=pl.ANY),
            out_shape=jax.ShapeDtypeStruct((R, D), x.dtype),
            scratch_shapes=[
                pltpu.VMEM((R, D), bf16),
                pltpu.VMEM((D, W), bf16),
                pltpu.VMEM((P, D, G * 128), bf16),
                pltpu.VMEM((P, D, G * 128), bf16),
                pltpu.VMEM((D, W), bf16),
                pltpu.VMEM((NBUF, P, Sk, Dh), bf16),
                pltpu.VMEM((NBUF, P, Sk, Dh), bf16),
                pltpu.VMEM((TPH, P * Sq, 128), bf16),
                pltpu.VMEM((NTL, R + 2 * pad, 128), bf16),
                pltpu.VMEM((NTL, R + pad, 128), f32),
                pltpu.VMEM((Hq, R + pad, 128), f32),
                pltpu.VMEM((TPH, P * Sq, 128), f32),
                pltpu.VMEM((rep, P * Sq, 128), f32),
                pltpu.VMEM((D, R), f32),
                pltpu.VMEM((R, D), bf16),
                pltpu.VMEM((P, M, Sk), f32),
                pltpu.VMEM((P, M, 128), f32),
                pltpu.VMEM((R // 128 - bar, 128, W), bf16),
                pltpu.VMEM((D, 128), bf16),
                pltpu.VMEM((max(nnorm, 1), 128, D), f32),
                pltpu.SemaphoreType.REGULAR,
                pltpu.SemaphoreType.DMA((NBUF,)),
                pltpu.SemaphoreType.DMA((NBUF,)),
                pltpu.SemaphoreType.DMA((P,)),
                pltpu.SemaphoreType.DMA((P,)),
                pltpu.SemaphoreType.DMA((4,)),
                pltpu.SemaphoreType.DMA((len(out_groups),)),
            ],
            compiler_params=pltpu.CompilerParams(
                vmem_limit_bytes=vmem * 1024 * 1024,
                disable_bounds_checks=not checks,
                disable_semaphore_checks=not checks,
            ),
        )(x2, k_cache, v_cache, wq, woT)
        return out.reshape(B, Sq, D)
    return fn


@jax.jit
def pallas_standalone__gqa_block_cached__near_ridge_kernel(x, k_cache, v_cache, wq, wo):
    return _make()(x, k_cache, v_cache, wq, wo)
```

```python
import functools
import jax
import jax.numpy as jnp
from jax import lax
import jax.experimental.pallas as pl
import jax.experimental.pallas.tpu as pltpu

LOG2E = 1.4426950408889634

def _make(KC=256, KCE=512, vmem=127, checks=False, xsplit=2, dma_at=0, nnorm=1, CU=2, amid=1, lag=2,
         pre=9, tdep=True, aearly=0, anchor=True, arows=4, arow=280, both=False, amode=1, cheat2=False, endmode='late', ai=3, ac=0, qanchor=None, rmw=True, amask='all', alag=0, hand='end', qrow=None, issue_ch=2, ngrp=12, grp0=0, wlay='tk', wpad=0, xpad=8, wdep=True):
    P = 4
    NBUF = 2
    def _recip(l):
        r = pl.reciprocal(l, approx=True)
        return r * (2.0 - l * r)

    def fn(x, k_cache, v_cache, wq, wo):
        B, Sq, D = x.shape
        _, Hkv, Sk, Dh = k_cache.shape
        Hq = wq.shape[1] // Dh
        rep = Hq // Hkv
        M = rep * Sq
        W = rep * Dh
        R = B * Sq
        TPH = W // 128
        TPQ = Dh // 128
        NTL = Hq * Dh // 128
        G = (NTL - TPH) // P
        assert G * P == NTL - TPH
        DM = (D // 128) * 128
        KR = D - DM
        scale = Dh ** -0.5 * LOG2E
        x2 = x.reshape(R, D)
        woT = wo.T
        NP = B * Hkv
        NS = NP // P
        SPH = B // P
        assert SPH == 2
        NT = (((1,), (1,)), ((), ()))
        f32, bf16, i32 = jnp.float32, jnp.bfloat16, jnp.int32
        XR = xsplit * Sq
        HR = P * Sq
        NO = R // 128
        bits = lambda v: lax.bitcast_convert_type(v, i32)
        flt = lambda v: lax.bitcast_convert_type(v, f32)

        def kernel(x_hbm, k_hbm, v_hbm, wq_hbm, wo_hbm, out_hbm,
                   x_v, wq0_v, wqr_v, kbuf, vbuf, q0, qs, qa, ou_all, l_all, ou7, l7,
                   accT, s_scr, m_scr, acc_n, xB, wf, mr_scr,
                   ksem, vsem, k0sem, wqsem, wsem, osem):
            wor_v, wo7_v, out_v = wqr_v, wq0_v, x_v
            def blk(t):
                if isinstance(t, int):
                    return t // SPH, (t % SPH) * P
                return lax.shift_right_logical(t, 1), (t & 1) * P
            def kcopy(t, slot):
                h, b0 = blk(t)
                return pltpu.make_async_copy(k_hbm.at[pl.ds(b0, P), h], kbuf.at[slot], ksem.at[slot])
            def vcopy(t, slot):
                h, b0 = blk(t)
                return pltpu.make_async_copy(v_hbm.at[pl.ds(b0, P), h], vbuf.at[slot], vsem.at[slot])
            def k0copy(i):
                return pltpu.make_async_copy(k_hbm.at[i, 0], kbuf.at[0, i], k0sem.at[i])
            xa = pltpu.make_async_copy(x_hbm.at[pl.ds(0, XR)], x_v.at[pl.ds(0, XR)], wsem.at[0])
            xb = pltpu.make_async_copy(x_hbm.at[pl.ds(XR, R - XR)], x_v.at[pl.ds(XR, R - XR)], wsem.at[1])
            wq0c = pltpu.make_async_copy(wq_hbm.at[:, pl.ds(0, W)], wq0_v, wsem.at[2])
            def wqrc(i):
                return pltpu.make_async_copy(wq_hbm.at[:, pl.ds(W + i * G * 128, G * 128)], wqr_v.at[i], wqsem.at[i])
            worc = [pltpu.make_async_copy(wo_hbm.at[:, pl.ds(i * G * 128, G * 128)], wor_v.at[i], wsem.at[3]) for i in range(P)]
            wo7c = pltpu.make_async_copy(wo_hbm.at[:, pl.ds(P * G * 128, W)], wo7_v, wsem.at[3])

            xa.start()
            wq0c.start()
            xb.start()
            accT[...] = jnp.zeros_like(accT)

            def qproj0(r0, r1):
                q = jnp.dot(x_v[r0:r1, :], wq0_v[...], preferred_element_type=f32)
                q = pltpu.bitcast((q * scale).astype(bf16), i32)
                for k in range(TPH):
                    for b in range(r0 // Sq, r1 // Sq):
                        val = q[(b * Sq - r0) // 2:((b + 1) * Sq - r0) // 2, k * 128:(k + 1) * 128]
                        if b < P:
                            q0[b, k] = val
                        else:
                            qs[b - P, k] = val

            xa.wait()
            wq0c.wait()
            k0copy(0).start()
            wqrc(0).start()
            qproj0(0, XR)
            xb.wait()
            k0copy(1).start()
            wqrc(1).start()
            qproj0(XR, R)

            def load_q(ref, i, dep=None, drow=0):
                qi = jnp.concatenate(
                    [jnp.concatenate([ref[i, r * TPQ + c] for c in range(TPQ)], axis=1) for r in range(rep)], axis=0)
                if dep is not None:
                    mid = jnp.concatenate([qi[drow:drow + 8, 0:128] | dep, qi[drow:drow + 8, 128:]], axis=1)
                    qi = jnp.concatenate([v for v in (qi[:drow], mid, qi[drow + 8:]) if v.shape[0]], axis=0)
                return pltpu.bitcast(qi, bf16)

            def sub(i, qk, pv, split_last, kc, hook=None, mem=None):
                edges = list(range(0, Sk + 1, kc))
                late = split_last and endmode == 'late'
                split_last = split_last and endmode == 'split'
                if split_last:
                    edges = [e for e in edges if e <= Sk - 512 or e == Sk]
                nc = len(edges) - 1
                mrun = None
                o = None
                l = None
                mx = None
                for j in range(nc):
                    last = j == nc - 1
                    k0_, k1_ = edges[j], edges[j + 1]
                    nt = (k1_ - k0_) // 128
                    ks = slice(k0_, k1_)
                    if pv is not None:
                        store_o, store_l, vslot = pv
                        m = m_scr[i]
                        pj = jnp.exp2(s_scr[i, :, ks] - jnp.concatenate([m] * nt, axis=1))
                        lj = None
                        for c in range(nt):
                            pc = pj[:, c * 128:(c + 1) * 128]
                            lj = pc if lj is None else lj + pc
                        if mem is not None:
                            load_o, load_l, zm = mem
                            store_l(lj if j == 0 else lj + load_l())
                            if j > 0:
                                o = load_o()
                        else:
                            l = lj if l is None else l + lj
                        pb = pj.astype(bf16)
                        if last and mem is None:
                            store_l(l)
                        if last and split_last:
                            oa = jnp.dot(pb, vbuf[vslot, i, ks, 0:128], preferred_element_type=f32)
                            store_o(0, oa + o[:, 0:128])
                        elif not (last and late):
                            oj = jnp.dot(pb, vbuf[vslot, i, ks, :], preferred_element_type=f32)
                            o = oj if o is None else oj + o
                            if last or mem is not None:
                                for c in range(TPQ):
                                    store_o(c, o[:, c * 128:(c + 1) * 128])
                    if hook is not None:
                        hook(nt)
                    if qk is not None:
                        getq, kslot = qk
                        for q0_ in range(k0_, k1_, kc):
                            qsl = slice(q0_, q0_ + kc)
                            s = lax.dot_general(getq(q0_), kbuf[kslot, i, qsl, :], NT, preferred_element_type=f32)
                            s_scr[i, :, qsl] = s
                            if mem is not None and q0_ > 0:
                                mrun = mr_scr[mem[2]]
                            for c in range(kc // 128):
                                sc = s[:, c * 128:(c + 1) * 128]
                                mrun = sc if mrun is None else jnp.maximum(mrun, sc)
                            if mem is not None and q0_ + kc < Sk:
                                mr_scr[mem[2]] = mrun
                            if hook is not None and q0_ + kc < k1_:
                                hook(kc // 128)
                        if last:
                            mx = jnp.broadcast_to(jnp.max(mrun, axis=-1, keepdims=True), (M, 128))
                            m_scr[i] = mx
                    if hook is not None:
                        hook(kc // 128)
                    if pv is not None and last and split_last:
                        ob = jnp.dot(pb, vbuf[vslot, i, ks, 128:256], preferred_element_type=f32)
                        if mem is not None:
                            o = mem[0]()
                        store_o(1, ob + o[:, 128:256])
                    if pv is not None and last and late:
                        o = jnp.dot(pb, vbuf[vslot, i, ks, :], preferred_element_type=f32) + (o if mem is None else mem[0]())
                        for c in range(TPQ):
                            store_o(c, o[:, c * 128:(c + 1) * 128])
                return mx

            TR = R // P
            def abody(i, zc):
                k0copy(i).wait()
                wqrc(i).wait()
                qfirst = []
                def qpart(g0, g1):
                    rg = R // arows
                    for g in range(g0, g1):
                        q = jnp.dot(x_v[g * rg:(g + 1) * rg, 0:DM], wqr_v[i, 0:DM, :], preferred_element_type=f32)
                        for k in range(G):
                            qa[i * G + k, g * rg:(g + 1) * rg, :] = q[:, k * 128:(k + 1) * 128]
                        qfirst.append(q)
                if amid:
                    qpart(0, amid)
                @pl.when(i + 2 < P)
                def _():
                    k0copy(i + 2).start()
                    wqrc(i + 2).start()
                @pl.when(i == 0)
                def _():
                    kcopy(1, 1).start()
                @pl.when(i == 1)
                def _():
                    vcopy(0, 0).start()
                mx = sub(i, (lambda c: load_q(q0, i), 0), None, False, KCE)
                qpart(amid, arows)
                rows = pl.ds(pl.multiple_of(i * TR, 16), TR)
                xr = x_v[rows, DM:D]
                if tdep:
                    xr = pltpu.bitcast(pltpu.bitcast(xr, i32)
                                       | (bits(mx[0:TR // 2, 0:KR]) & jnp.full((TR // 2, KR), zc[0] * zc[1], i32)), bf16)
                xr = xr.astype(f32)
                for kk in range(KR):
                    xB[kk, rows, :] = jnp.broadcast_to(xr[:, kk:kk + 1], (TR, 128))
                wr = wqr_v[i, DM:D, :].astype(f32)
                if wlay == 'perm':
                    for k in range(G):
                        wf[i * G + k] = wr[:, k * 128:(k + 1) * 128]
                else:
                  for kk in range(KR):
                    wrow = jnp.broadcast_to(wr[kk:kk + 1, :], (8, G * 128))
                    if wdep:
                        nrg = R // arows // 8
                        n_ = kk * (nrg * G) // KR
                        src_ = qfirst[0][(n_ % nrg) * 8:(n_ % nrg) * 8 + 8, (n_ // nrg) * 128:(n_ // nrg + 1) * 128]
                        d_ = bits(src_) & jnp.full((8, 128), zc[0] * zc[1], i32)
                        wrow = flt(bits(wrow) | jnp.concatenate([d_] * G, axis=1))
                    for k in range(G):
                        if wlay == 'tk':
                            wf[i * G + k, kk] = wrow[:, k * 128:(k + 1) * 128]
                        else:
                            wf[kk, i * G + k] = wrow[:, k * 128:(k + 1) * 128]
                return (zc[1], zc[0])
            lax.fori_loop(0, P, abody, (jnp.int32(0), jnp.int32(1)))

            def body(t, slots):
                sm1, s0 = slots
                tn = jnp.minimum(t + 1, NS - 1)
                kcopy(t, s0).wait()
                vcopy(t - 1, sm1).wait()
                hp, bp0 = blk(t - 1)
                hn, bn0 = blk(tn)
                z1 = sm1 * s0
                z2 = sm1 + s0 - 1
                zvec = jnp.full((8, 128), z1, i32)
                def issue():
                    @pl.when(t + 1 < NS)
                    def _():
                        kcopy(t + 1, sm1).start()
                    vcopy(t, s0).start()
                    @pl.when(t == NS - 2)
                    def _():
                        for cc in worc:
                            cc.start()
                        wo7c.start()
                if hand == 'shift':
                    NRG = Sq // 16
                    pieces = [((i + P - 1) % P, (n % NRG) * 16, n % TPH) for i in range(P) for n in range(NRG * TPH)]
                    for k_ in range(TPH):
                        q0[z1, k_] = qs[P - 1, k_]
                else:
                    RGS = [(i, r0) for i in range(P) for r0 in range(0, Sq, 16)]
                    pieces = [RGS[n % len(RGS)] + ((n + n // len(RGS)) % TPH,) for n in range(len(RGS) * TPH)]
                assert len(set(pieces)) == len(pieces)
                st = dict(n=0, ch=0, prev=None)
                done = []
                hist = []
                def piece():
                    i, r0, ct = pieces[st['n']]
                    st['n'] += 1
                    rows = pl.ds(pl.multiple_of((bn0 + i) * Sq + r0, 16), 16)
                    acc = qa[(hn - 1) * TPH + ct, rows, :]
                    for kk in range(KR):
                        if kk == pre and st['prev'] is not None:
                            dep = st['prev'] & zvec
                            acc = flt(bits(acc) | jnp.concatenate([dep, dep], axis=0))
                        if wlay == 'perm':
                            if kk % 8 == 0:
                                w8 = wf[(hn - 1) * TPH + ct, kk:kk + 8, :]
                            wk = jnp.broadcast_to(w8[kk % 8:kk % 8 + 1, :], (8, 128))
                        else:
                            wk = wf[(hn - 1) * TPH + ct, kk] if wlay == 'tk' else wf[kk, (hn - 1) * TPH + ct]
                        acc = acc + xB[kk, rows, :] * jnp.concatenate([wk, wk], axis=0)
                    st['prev'] = pltpu.bitcast((acc * scale).astype(bf16), i32)
                    hist.append(st['prev'])
                    if hand == 'shift':
                        qs[i, ct, r0 // 2:r0 // 2 + 8, :] = st['prev']
                    elif cheat2:
                        q0[i, ct, r0 // 2:r0 // 2 + 8, :] = st['prev']
                    else:
                        done.append((i, r0, ct, st['prev']))
                nh = 2 * (Sk // 128) * P - aearly
                def hook(nt):
                    st['ch'] += nt
                    while st['n'] < min(len(pieces), len(pieces) * st['ch'] // nh):
                        piece()
                    if st['ch'] == issue_ch:
                        issue()
                    if st['ch'] == 2 * (Sk // 128) * P and qrow is None and not ngrp:
                        for i, r0, ct, val in done:
                            qs[i + z1, ct, r0 // 2:r0 // 2 + 8, :] = val
                for i in range(P):
                    if i == 0 and issue_ch == 0:
                        issue()
                    row = pl.multiple_of((bp0 + i) * Sq, 16)
                    def store_o(c, val, row=row, i=i):
                        fin_ = st['n'] == len(pieces)
                        if anchor and c == ac and (fin_ or amask == 'all' or (amask == 'pair' and i == P - 1)) and len(hist) > alag:
                            back = hist[-1] if fin_ else hist[-1 - alag]
                            mid = flt(bits(val[arow:arow + 8]) | (back & zvec))
                            val = jnp.concatenate([v for v in (val[:arow], mid, val[arow + 8:]) if v.shape[0]], axis=0)
                        if qrow is not None and fin_ and c == 0:
                            mid = flt(bits(val[qrow:qrow + 8]) | (qs[z2, 0, 0:8, :] & zvec))
                            val = jnp.concatenate([v for v in (val[:qrow], mid, val[qrow + 8:]) if v.shape[0]], axis=0)
                        if ngrp and fin_ and c == 0:
                            step = (M - grp0) // 8 // ngrp * 8
                            per = len(done) // ngrp
                            parts = [val[:grp0]] if grp0 else []
                            for g in range(ngrp):
                                a = grp0 + g * step
                                b = M if g == ngrp - 1 else a + step
                                parts.append(flt(bits(val[a:a + 8]) | (qs[z2, 0, 0:8, :] & zvec)))
                                if b > a + 8:
                                    parts.append(val[a + 8:b])
                                for i_, r0, ct, v_ in done[g * per:(g + 1) * per]:
                                    qs[i_ + z1, ct, r0 // 2:r0 // 2 + 8, :] = v_
                            val = jnp.concatenate(parts, axis=0)
                        for r in range(rep):
                            ou_all[hp * TPH + r * TPQ + c, pl.ds(row, Sq), :] = val[r * Sq:(r + 1) * Sq]
                    def store_l(val, row=row):
                        for r in range(rep):
                            l_all[hp * rep + r, pl.ds(row, Sq), :] = val[r * Sq:(r + 1) * Sq]
                    def load_o(row=row):
                        return jnp.concatenate([jnp.concatenate(
                            [ou_all[hp * TPH + r * TPQ + c, pl.ds(row, Sq), :] for c in range(TPQ)], axis=1)
                            for r in range(rep)], axis=0)
                    def load_l(row=row):
                        return jnp.concatenate([l_all[hp * rep + r, pl.ds(row, Sq), :] for r in range(rep)], axis=0)
                    sub(i, (lambda c, i=i: load_q(q0, z1) if (hand == 'shift' and i == P - 1) else load_q(qs, i), s0), (store_o, store_l, sm1), i == P - 1, KC, hook, (load_o, load_l, z1) if rmw else None)
                if qrow is not None:
                    for i, r0, ct, val in done:
                        qs[i + z1, ct, r0 // 2:r0 // 2 + 8, :] = val
                return (s0, sm1)
            fin = lax.fori_loop(1, NS, body, (jnp.int32(0), jnp.int32(1)))
            zero = fin[0] * fin[1]

            vlast = (NS - 1) % NBUF
            if cheat2:
                m_scr[0, 0:72] = m_scr[0, 0:72] + sum(flt(q0[a, b]) for a in range(P) for b in range(TPH))
            vcopy(NS - 1, vlast).wait()
            for cc in worc:
                cc.wait()
            wo7c.wait()
            def cbody(ii, c):
                for u in range(CU):
                    i = ii * CU + u
                    row = pl.multiple_of(i * Sq, 16)
                    def store_o(cc, val, row=row):
                        for r in range(rep):
                            ou7[r * TPQ + cc, pl.ds(row, Sq), :] = val[r * Sq:(r + 1) * Sq]
                    def store_l(val, row=row):
                        for r in range(rep):
                            l7[r, pl.ds(row, Sq), :] = val[r * Sq:(r + 1) * Sq]
                    sub(i, None, (store_o, store_l, vlast), False, KCE)
                tiles = []
                for k2 in range(CU * G // 2):
                    kq = ii * (CU * G // 2) + k2
                    rc = _recip(jnp.sum(l_all[kq], axis=-1, keepdims=True))
                    for cc in range(TPQ):
                        tiles.append(ou_all[kq * TPQ + cc] * rc)
                on = jnp.concatenate(tiles, axis=1).astype(bf16)
                w = jnp.concatenate([wor_v[ii * CU + u] for u in range(CU)], axis=1)
                accT[...] += lax.dot_general(w, on, NT, preferred_element_type=f32)
                return c
            lax.fori_loop(0, P // CU, cbody, 0)

            def rows_of(big, small, idx_big, idx_small, r0, r1):
                parts = []
                if r0 < HR:
                    parts.append(big[idx_big, r0:min(r1, HR), :])
                if r1 > HR:
                    parts.append(small[idx_small, max(r0, HR) - HR:r1 - HR, :])
                return parts[0] if len(parts) == 1 else jnp.concatenate(parts, axis=0)
            ocs = []
            def emit(n, res):
                r0 = n * 128
                out_v[pl.ds(pl.multiple_of(r0 + zero, 128), 128), :] = res
                oc = pltpu.make_async_copy(out_v.at[pl.ds(r0, 128)], out_hbm.at[pl.ds(r0, 128)], osem.at[n])
                oc.start()
                ocs.append(oc)
            def normed7(n):
                r0, r1 = n * 128, (n + 1) * 128
                tiles = []
                for r in range(rep):
                    l = jnp.sum(rows_of(l_all, l7, (Hkv - 1) * rep + r, r, r0, r1), axis=-1, keepdims=True)
                    rc = _recip(l)
                    for cc in range(TPQ):
                        tiles.append(rows_of(ou_all, ou7, (Hkv - 1) * TPH + r * TPQ + cc, r * TPQ + cc, r0, r1) * rc)
                return jnp.concatenate(tiles, axis=1).astype(bf16)
            for n in range(NO - nnorm, NO):
                acc_n[n - NO + nnorm] = accT[:, n * 128:(n + 1) * 128].T
            res = {}
            for n in range(NO + lag):
                if n >= lag:
                    emit(n - lag, res.pop(n - lag))
                if n >= NO:
                    continue
                r0, r1 = n * 128, (n + 1) * 128
                on = normed7(n)
                if n >= lag:
                    rows = pl.ds(pl.multiple_of(r0 + zero, 128), 128)
                    out_v[rows, 0:128] = on[:, 0:128]
                    on = jnp.concatenate([out_v[rows, 0:128], on[:, 128:]], axis=1)
                if n >= NO - nnorm:
                    res[n] = (lax.dot_general(on, wo7_v[...], NT, preferred_element_type=f32) + acc_n[n - NO + nnorm]).astype(bf16)
                else:
                    res[n] = (lax.dot_general(wo7_v[...], on, NT, preferred_element_type=f32) + accT[:, r0:r1]).astype(bf16).T
            for oc in ocs:
                oc.wait()

        out = pl.pallas_call(
            kernel,
            in_specs=[pl.BlockSpec(memory_space=pl.ANY)] * 5,
            out_specs=pl.BlockSpec(memory_space=pl.ANY),
            out_shape=jax.ShapeDtypeStruct((R, D), x.dtype),
            scratch_shapes=[
                pltpu.VMEM((R, D), bf16),
                pltpu.VMEM((D, W), bf16),
                pltpu.VMEM((P, D, G * 128), bf16),
                pltpu.VMEM((NBUF, P, Sk, Dh), bf16),
                pltpu.VMEM((NBUF, P, Sk, Dh), bf16),
                pltpu.VMEM((P, TPH, Sq // 2, 128), i32),
                pltpu.VMEM((P, TPH, Sq // 2, 128), i32),
                pltpu.VMEM((NTL - TPH, R, 128), f32),
                pltpu.VMEM((NTL, R, 128), f32),
                pltpu.VMEM((Hq, R, 128), f32),
                pltpu.VMEM((TPH, P * Sq, 128), f32),
                pltpu.VMEM((rep, P * Sq, 128), f32),
                pltpu.VMEM((D, R), f32),
                pltpu.VMEM((P, M, Sk), f32),
                pltpu.VMEM((P, M, 128), f32),
                pltpu.VMEM((max(nnorm, 1), 128, D), f32),
                pltpu.VMEM((KR, R + xpad, 128), f32),
                pltpu.VMEM({'tk': (NTL - TPH, KR + wpad, 8, 128), 'kt': (KR, NTL - TPH + wpad, 8, 128), 'perm': (NTL - TPH, KR, 128)}[wlay], f32),
                pltpu.VMEM((2, M, 128), f32),
                pltpu.SemaphoreType.DMA((NBUF,)),
                pltpu.SemaphoreType.DMA((NBUF,)),
                pltpu.SemaphoreType.DMA((P,)),
                pltpu.SemaphoreType.DMA((P,)),
                pltpu.SemaphoreType.DMA((4,)),
                pltpu.SemaphoreType.DMA((NO,)),
            ],
            compiler_params=pltpu.CompilerParams(
                vmem_limit_bytes=vmem * 1024 * 1024,
                disable_bounds_checks=not checks,
                disable_semaphore_checks=not checks,
            ),
        )(x2, k_cache, v_cache, wq, woT)
        return out.reshape(B, Sq, D)
    return fn


@jax.jit
def pallas_standalone__gqa_block_cached__near_ridge_kernel(x, k_cache, v_cache, wq, wo):
    return _make()(x, k_cache, v_cache, wq, wo)
```

```python
import jax
import jax.numpy as jnp
from jax import lax
import jax.experimental.pallas as pl
import jax.experimental.pallas.tpu as pltpu

LOG2E = 1.4426950408889634
f32, bf16, i32 = jnp.float32, jnp.bfloat16, jnp.int32
NT = (((1,), (1,)), ((), ()))


def _bits(v):
    return lax.bitcast_convert_type(v, i32)


def _flt(v):
    return lax.bitcast_convert_type(v, f32)


def _recip(l):
    r = pl.reciprocal(l, approx=True)
    return r * (2.0 - l * r)


def _tie(val, row, dep):
    parts = [val[:row]] if row else []
    parts.append(_flt(_bits(val[row:row + 8]) | dep))
    if row + 8 < val.shape[0]:
        parts.append(val[row + 8:])
    return jnp.concatenate(parts, axis=0)


def _make(KC=256, KCE=512, vmem=127, checks=False, xsplit=2, CU=2, arows=4, lag=2,
         pre=8, ngrp=12, gs=8, lead=32, delta=125.0):
    P = 4

    def fn(x, k_cache, v_cache, wq, wo):
        B, Sq, D = x.shape
        _, Hkv, Sk, Dh = k_cache.shape
        Hq = wq.shape[1] // Dh
        rep = Hq // Hkv
        M = rep * Sq
        W = rep * Dh
        R = B * Sq
        TPH = W // 128
        TPQ = Dh // 128
        NTL = Hq * Dh // 128
        G = (NTL - TPH) // P
        DM = (D // 128) * 128
        KR = D - DM
        NS = B * Hkv // P
        HR = P * Sq
        NO = R // 128
        XR = xsplit * Sq
        TR = R // P
        assert G * P == NTL - TPH and B == 2 * P and R % 128 == 0 and Sq % 16 == 0 and TR % 16 == 0
        assert KR % gs == 0 and pre % gs == 0 and (CU * G) % TPQ == 0
        scale = Dh ** -0.5 * LOG2E

        def kernel(x_hbm, k_hbm, v_hbm, wq_hbm, wo_hbm, out_hbm,
                   x_v, wq0_v, wqr_v, vbuf, ou_all, l_all, s_scr, m_scr,
                   ksem, vsem, k0sem, wqsem, wsem, osem):
            wor_v, wo7_v, out_v = wqr_v, wq0_v, x_v

            def blk(t):
                if isinstance(t, int):
                    return t // 2, (t % 2) * P
                return lax.shift_right_logical(t, 1), (t & 1) * P

            def vcopy(t, slot):
                h, b0 = blk(t)
                return pltpu.make_async_copy(v_hbm.at[pl.ds(b0, P), h], vbuf.at[slot], vsem.at[slot])

            wocs = [pltpu.make_async_copy(wo_hbm.at[:, pl.ds(i * G * 128, G * 128)], wor_v.at[i], wsem.at[3])
                    for i in range(P)]
            wocs.append(pltpu.make_async_copy(wo_hbm.at[:, pl.ds(P * G * 128, W)], wo7_v, wsem.at[3]))

            def probs(i, ks):
                nt = (ks.stop - ks.start) // 128
                p = jnp.exp2(s_scr[i, :, ks] - jnp.concatenate([m_scr[i]] * nt, axis=1))
                l = p[:, 0:128]
                for c in range(1, nt):
                    l = l + p[:, c * 128:(c + 1) * 128]
                return p.astype(bf16), l

            def front(kbuf, q0, qs, qa, mr_scr, xB, wB):
                def kcopy(t, slot):
                    h, b0 = blk(t)
                    return pltpu.make_async_copy(k_hbm.at[pl.ds(b0, P), h], kbuf.at[slot], ksem.at[slot])

                def k0copy(i):
                    return pltpu.make_async_copy(k_hbm.at[i, 0], kbuf.at[0, i], k0sem.at[i])

                def wqrc(i):
                    return pltpu.make_async_copy(
                        wq_hbm.at[:, pl.ds(W + i * G * 128, G * 128)], wqr_v.at[i], wqsem.at[i])

                xa = pltpu.make_async_copy(x_hbm.at[pl.ds(0, XR)], x_v.at[pl.ds(0, XR)], wsem.at[0])
                xb = pltpu.make_async_copy(x_hbm.at[pl.ds(XR, R - XR)], x_v.at[pl.ds(XR, R - XR)], wsem.at[1])
                wq0c = pltpu.make_async_copy(wq_hbm.at[:, pl.ds(0, W)], wq0_v, wsem.at[2])

                def qproj0(r0, r1):
                    q = jnp.dot(x_v[r0:r1, :], wq0_v[...], preferred_element_type=f32)
                    q = pltpu.bitcast((q * scale).astype(bf16), i32)
                    for b in range(r0 // Sq, r1 // Sq):
                        qb = q[(b * Sq - r0) // 2:((b + 1) * Sq - r0) // 2]
                        val = jnp.stack([qb[:, k * 128:(k + 1) * 128] for k in range(TPH)])
                        if b < P:
                            q0[b] = val
                        else:
                            qs[b - P] = val

                xa.start()
                wq0c.start()
                xb.start()
                xa.wait()
                wq0c.wait()
                k0copy(0).start()
                wqrc(0).start()
                qproj0(0, XR)
                xb.wait()
                k0copy(1).start()
                wqrc(1).start()
                qproj0(XR, R)

                def load_q(ref, i):
                    q = ref[i]
                    return pltpu.bitcast(jnp.concatenate(
                        [jnp.concatenate([q[r * TPQ + c] for c in range(TPQ)], axis=1) for r in range(rep)],
                        axis=0), bf16)

                def colmax(s, mrun):
                    for c in range(s.shape[1] // 128):
                        sc = s[:, c * 128:(c + 1) * 128]
                        mrun = sc if mrun is None else jnp.maximum(mrun, sc)
                    return mrun

                def rowmax(mrun):
                    return jnp.broadcast_to(jnp.max(mrun, axis=-1, keepdims=True), (M, 128))

                def abody(i, zc):
                    k0copy(i).wait()
                    wqrc(i).wait()
                    zv = jnp.full((8, 128), zc[0] * zc[1], i32)
                    rg = R // arows

                    @pl.when(i + 2 < P)
                    def _():
                        wqrc(i + 2).start()

                    @pl.when(i + 2 < P)
                    def _():
                        k0copy(i + 2).start()

                    @pl.when(i == 0)
                    def _():
                        kcopy(1, 1).start()

                    @pl.when(i == 1)
                    def _():
                        vcopy(0, 0).start()

                    def qpart(g):
                        q = jnp.dot(x_v[g * rg:(g + 1) * rg, 0:DM], wqr_v[i, 0:DM, :], preferred_element_type=f32)
                        q = q * scale
                        qa[pl.ds(i * G, G), g * rg // 8:(g + 1) * rg // 8] = jnp.stack(
                            [q[:, k * 128:(k + 1) * 128].reshape(rg // 8, 8, 128) for k in range(G)])
                        return q

                    qp = qpart(0)
                    mrun = None
                    for k0 in range(0, Sk, KCE):
                        s = lax.dot_general(load_q(q0, i), kbuf[0, i, k0:k0 + KCE, :], NT,
                                            preferred_element_type=f32)
                        s_scr[i, :, k0:k0 + KCE] = s
                        mrun = colmax(s, mrun)
                    mx = rowmax(mrun)
                    m_scr[i] = mx
                    for g in range(1, arows):
                        qpart(g)

                    dep = _bits(mx[M - 8:M])
                    for u in range(2, M // 8 + 1):
                        dep = dep | _bits(mx[M - 8 * u:M - 8 * u + 8])
                    dep = jnp.concatenate([(dep & zv)[:, 0:KR]] * (TR // 16), axis=0)
                    xr = x_v[pl.ds(pl.multiple_of(i * TR, 16), TR), DM:D]
                    xr = pltpu.bitcast(pltpu.bitcast(xr, i32) | dep, bf16).astype(f32)
                    xB[:, pl.ds(i * (TR // 8), TR // 8)] = jnp.stack(
                        [jnp.broadcast_to(xr[:, kk:kk + 1], (TR, 128)).reshape(TR // 8, 8, 128) for kk in range(KR)])
                    wr = wqr_v[i, DM:D, :].astype(f32) * scale
                    nrg = rg // 8
                    wrows = []
                    for kk in range(KR):
                        n = kk * (nrg * G) // KR
                        dep = _bits(qp[(n % nrg) * 8:(n % nrg) * 8 + 8, (n // nrg) * 128:(n // nrg + 1) * 128]) & zv
                        wrow = jnp.broadcast_to(wr[kk:kk + 1, :], (8, G * 128))
                        wrows.append(_flt(_bits(wrow) | jnp.concatenate([dep] * G, axis=1)))
                    wall = jnp.stack(wrows)
                    wB[pl.ds(i * G, G)] = jnp.stack([wall[:, :, k * 128:(k + 1) * 128] for k in range(G)])
                    return (zc[1], zc[0])

                lax.fori_loop(0, P, abody, (jnp.int32(0), jnp.int32(1)))

                NC = Sk // KC
                RGS = [(i, r0) for i in range(P) for r0 in range(0, Sq, 16)]
                pieces = [RGS[n % len(RGS)] + ((n + n // len(RGS)) % TPH,) for n in range(len(RGS) * TPH)]
                assert len(set(pieces)) == len(pieces)
                due = [2 * NC * P * M - lead - (len(pieces) - 1 - n) * delta for n in range(len(pieces))]

                def body(t, slots):
                    sm1, s0 = slots
                    kcopy(t, s0).wait()
                    vcopy(t - 1, sm1).wait()
                    hp, bp0 = blk(t - 1)
                    hn, bn0 = blk(jnp.minimum(t + 1, NS - 1))
                    z1 = sm1 * s0
                    z2 = sm1 + s0 - 1
                    zvec = jnp.full((8, 128), z1, i32)
                    wt = [(hn - 1) * TPH + ct for ct in range(TPH)]
                    otile = pl.ds(hp * TPH, TPH)
                    ltile = pl.ds(hp * rep, rep)
                    rg0 = bn0 * (Sq // 8)
                    done = []
                    nmm = [0]

                    def piece():
                        i, r0, ct = pieces[len(done)]
                        rows = pl.ds(rg0 + (i * Sq + r0) // 8, 2)
                        acc = qa[wt[ct], rows][None]
                        for k0 in range(0, KR, gs):
                            xg = xB[k0:k0 + gs, rows]
                            wg = wB[wt[ct], k0:k0 + gs][:, None]
                            if k0 == pre and done:
                                acc = _flt(_bits(acc) | (done[-1] & zvec)[None, None])
                            prod = xg * wg
                            for u in range(gs):
                                acc = acc + prod[u:u + 1]
                        done.append(pltpu.bitcast(acc.reshape(16, 128).astype(bf16), i32))

                    def paced(val):
                        c = nmm[0]
                        nmm[0] += 1
                        while len(done) < len(pieces) and due[len(done)] < (c + 1) * M:
                            row = max(0, int(due[len(done)] - c * M)) // 8 * 8
                            piece()
                            val = _tie(val, row, done[-1] & zvec)
                        return val

                    for i in range(P):
                        rows = pl.ds(pl.multiple_of((bp0 + i) * Sq, 16), Sq)

                        def pv(j, pb, last):
                            o = jnp.dot(pb, vbuf[sm1, i, j * KC:(j + 1) * KC, :], preferred_element_type=f32)
                            if j > 0:
                                op = ou_all[otile, rows, :]
                                o = o + jnp.concatenate([jnp.concatenate(
                                    [op[r * TPQ + c] for c in range(TPQ)], axis=1) for r in range(rep)], axis=0)
                            vals = [o[:, c * 128:(c + 1) * 128] for c in range(TPQ)]
                            vals[0] = paced(vals[0])
                            if last:
                                res = dict(zip(pieces, done, strict=True))
                                step = M // 8 // ngrp * 8
                                per = len(RGS) // ngrp
                                for g in range(ngrp):
                                    vals[0] = _tie(vals[0], g * step, qs[z2, 0, 0:8, :] & zvec)
                                    grp = RGS[g * per:(g + 1) * per]
                                    pi, r0 = grp[0]
                                    assert grp[-1][0] == pi
                                    qs[pi + z1, :, r0 // 2:r0 // 2 + 8 * per, :] = jnp.stack(
                                        [jnp.concatenate([res[rg_ + (ct,)] for rg_ in grp], axis=0)
                                         for ct in range(TPH)])
                            ou_all[otile, rows, :] = jnp.stack(
                                [vals[c][r * Sq:(r + 1) * Sq] for r in range(rep) for c in range(TPQ)])

                        for j in range(NC):
                            ks = slice(j * KC, (j + 1) * KC)
                            last = i == P - 1 and j == NC - 1
                            pb, l = probs(i, ks)
                            l = l.reshape(rep, Sq, 128)
                            if j > 0:
                                l = l + l_all[ltile, rows, :]
                            l_all[ltile, rows, :] = l
                            if not last:
                                pv(j, pb, False)
                            if i == 0 and j == 0:
                                @pl.when(t + 1 < NS)
                                def _():
                                    kcopy(t + 1, sm1).start()

                                vcopy(t, s0).start()

                                @pl.when(t == NS - 2)
                                def _():
                                    for cc in wocs:
                                        cc.start()
                            s = lax.dot_general(load_q(qs, i), kbuf[s0, i, ks, :], NT, preferred_element_type=f32)
                            s_scr[i, :, ks] = jnp.concatenate([paced(s[:, 0:128]), s[:, 128:]], axis=1)
                            mrun = colmax(s, mr_scr[z1] if j > 0 else None)
                            if j < NC - 1:
                                mr_scr[z1] = mrun
                            else:
                                m_scr[i] = rowmax(mrun)
                            if last:
                                pv(j, pb, True)
                    return (s0, sm1)

                fin = lax.fori_loop(1, NS, body, (jnp.int32(0), jnp.int32(1)))
                return fin[0] * fin[1]

            zero = pl.run_scoped(
                front,
                pltpu.VMEM((2, P, Sk, Dh), bf16),
                pltpu.VMEM((P, TPH, Sq // 2, 128), i32),
                pltpu.VMEM((P, TPH, Sq // 2, 128), i32),
                pltpu.VMEM((NTL - TPH, R // 8, 8, 128), f32),
                pltpu.VMEM((2, M, 128), f32),
                pltpu.VMEM((KR, R // 8 + 1, 8, 128), f32),
                pltpu.VMEM((NTL - TPH, KR, 8, 128), f32),
            )

            def back(ou7, l7, accT, acc_n, on0):
                def rows_of(big, small, idx_big, idx_small, r0, r1):
                    parts = []
                    if r0 < HR:
                        parts.append(big[idx_big, r0:min(r1, HR), :])
                    if r1 > HR:
                        parts.append(small[idx_small, max(r0, HR) - HR:r1 - HR, :])
                    return parts[0] if len(parts) == 1 else jnp.concatenate(parts, axis=0)

                def normed7(n):
                    r0, r1 = n * 128, (n + 1) * 128
                    tiles = []
                    for r in range(rep):
                        l = jnp.sum(rows_of(l_all, l7, (Hkv - 1) * rep + r, r, r0, r1), axis=-1, keepdims=True)
                        rc = _recip(l)
                        for cc in range(TPQ):
                            k = r * TPQ + cc
                            tiles.append(rows_of(ou_all, ou7, (Hkv - 1) * TPH + k, k, r0, r1) * rc)
                    return jnp.concatenate(tiles, axis=1).astype(bf16)

                vlast = (NS - 1) % 2
                vcopy(NS - 1, vlast).wait()
                for cc in wocs:
                    cc.wait()

                def cbody(ii, c):
                    for u in range(CU):
                        i = ii * CU + u
                        rows = pl.ds(pl.multiple_of(i * Sq, 16), Sq)
                        o = None
                        l = None
                        for k0 in range(0, Sk, KCE):
                            pb, lj = probs(i, slice(k0, k0 + KCE))
                            l = lj if l is None else l + lj
                            if k0 + KCE == Sk:
                                l7[:, rows, :] = l.reshape(rep, Sq, 128)
                            oj = jnp.dot(pb, vbuf[vlast, i, k0:k0 + KCE, :], preferred_element_type=f32)
                            o = oj if o is None else oj + o
                        ou7[:, rows, :] = jnp.stack(
                            [o[r * Sq:(r + 1) * Sq, cc * 128:(cc + 1) * 128] for r in range(rep) for cc in range(TPQ)])
                    tiles = []
                    for k2 in range(CU * G // TPQ):
                        kq = ii * (CU * G // TPQ) + k2
                        rc = _recip(jnp.sum(l_all[kq], axis=-1, keepdims=True))
                        for cc in range(TPQ):
                            tiles.append(ou_all[kq * TPQ + cc] * rc)
                    on = jnp.concatenate(tiles, axis=1).astype(bf16)
                    w = jnp.concatenate([wor_v[ii * CU + u] for u in range(CU)], axis=1)
                    y = lax.dot_general(w, on, NT, preferred_element_type=f32) + jnp.where(ii > 0, accT[...], 0.0)
                    on0[...] = pltpu.bitcast(normed7(0), i32)
                    accT[...] = y
                    return c

                lax.fori_loop(0, P // CU, cbody, 0)

                acc_n[...] = accT[:, R - 128:R].T
                ocs = []
                res = {}
                for n in range(NO + lag):
                    if n >= lag:
                        r0 = (n - lag) * 128
                        out_v[pl.ds(pl.multiple_of(r0 + zero, 128), 128), :] = res.pop(n - lag)
                        oc = pltpu.make_async_copy(
                            out_v.at[pl.ds(r0, 128)], out_hbm.at[pl.ds(r0, 128)], osem.at[n - lag])
                        oc.start()
                        ocs.append(oc)
                    if n >= NO:
                        continue
                    r0, r1 = n * 128, (n + 1) * 128
                    on = normed7(n) if n > 0 else pltpu.bitcast(on0[...], bf16)
                    if n >= lag:
                        rows = pl.ds(pl.multiple_of(r0 + zero, 128), 128)
                        out_v[rows, 0:128] = on[:, 0:128]
                        on = jnp.concatenate([out_v[rows, 0:128], on[:, 128:]], axis=1)
                    if n == NO - 1:
                        res[n] = (lax.dot_general(on, wo7_v[...], NT, preferred_element_type=f32)
                                  + acc_n[...]).astype(bf16)
                    else:
                        res[n] = (lax.dot_general(wo7_v[...], on, NT, preferred_element_type=f32)
                                  + accT[:, r0:r1]).astype(bf16).T
                for oc in ocs:
                    oc.wait()

            pl.run_scoped(
                back,
                pltpu.VMEM((TPH, HR, 128), f32),
                pltpu.VMEM((rep, HR, 128), f32),
                pltpu.VMEM((D, R), f32),
                pltpu.VMEM((128, D), f32),
                pltpu.VMEM((64, W), i32),
            )

        out = pl.pallas_call(
            kernel,
            in_specs=[pl.BlockSpec(memory_space=pl.ANY)] * 5,
            out_specs=pl.BlockSpec(memory_space=pl.ANY),
            out_shape=jax.ShapeDtypeStruct((R, D), x.dtype),
            scratch_shapes=[
                pltpu.VMEM((R, D), bf16),
                pltpu.VMEM((D, W), bf16),
                pltpu.VMEM((P, D, G * 128), bf16),
                pltpu.VMEM((2, P, Sk, Dh), bf16),
                pltpu.VMEM((NTL, R, 128), f32),
                pltpu.VMEM((Hq, R, 128), f32),
                pltpu.VMEM((P, M, Sk), f32),
                pltpu.VMEM((P, M, 128), f32),
                pltpu.SemaphoreType.DMA((2,)),
                pltpu.SemaphoreType.DMA((2,)),
                pltpu.SemaphoreType.DMA((P,)),
                pltpu.SemaphoreType.DMA((P,)),
                pltpu.SemaphoreType.DMA((4,)),
                pltpu.SemaphoreType.DMA((NO,)),
            ],
            compiler_params=pltpu.CompilerParams(
                vmem_limit_bytes=vmem * 1024 * 1024,
                disable_bounds_checks=not checks,
                disable_semaphore_checks=not checks,
            ),
        )(x.reshape(R, D), k_cache, v_cache, wq, wo.T)
        return out.reshape(B, Sq, D)
    return fn


@jax.jit
def pallas_standalone__gqa_block_cached__near_ridge_kernel(
    x: jax.Array,
    k_cache: jax.Array,
    v_cache: jax.Array,
    wq: jax.Array,
    wo: jax.Array,
):
    return _make()(x, k_cache, v_cache, wq, wo)
```

```python
import jax
import jax.numpy as jnp
from jax import lax
import jax.experimental.pallas as pl
import jax.experimental.pallas.tpu as pltpu

LOG2E = 1.4426950408889634
f32, bf16, i32 = jnp.float32, jnp.bfloat16, jnp.int32
NT = (((1,), (1,)), ((), ()))


def _bits(v):
    return lax.bitcast_convert_type(v, i32)


def _flt(v):
    return lax.bitcast_convert_type(v, f32)


def _recip(l):
    r = pl.reciprocal(l, approx=True)
    return r * (2.0 - l * r)


def _tie(val, row, dep):
    parts = [val[:row]] if row else []
    parts.append(_flt(_bits(val[row:row + 8]) | dep))
    if row + 8 < val.shape[0]:
        parts.append(val[row + 8:])
    return jnp.concatenate(parts, axis=0)


def _make(KC=256, KCE=512, vmem=127, checks=False, xsplit=2, CU=2, arows=4, lag=2,
         pre=8, ngrp=12, gs=8, lead=32, delta=125.0, npre=4):
    P = 4

    def fn(x, k_cache, v_cache, wq, wo):
        B, Sq, D = x.shape
        _, Hkv, Sk, Dh = k_cache.shape
        Hq = wq.shape[1] // Dh
        rep = Hq // Hkv
        M = rep * Sq
        W = rep * Dh
        R = B * Sq
        TPH = W // 128
        TPQ = Dh // 128
        NTL = Hq * Dh // 128
        G = (NTL - TPH) // P
        DM = (D // 128) * 128
        KR = D - DM
        NS = B * Hkv // P
        HR = P * Sq
        NO = R // 128
        XR = xsplit * Sq
        TR = R // P
        assert G * P == NTL - TPH and B == 2 * P and R % 128 == 0 and Sq % 16 == 0 and TR % 16 == 0
        assert KR % gs == 0 and pre % gs == 0 and (CU * G) % TPQ == 0
        scale = Dh ** -0.5 * LOG2E

        def kernel(x_hbm, k_hbm, v_hbm, wq_hbm, wo_hbm, out_hbm,
                   x_v, wq0_v, wqr_v, vbuf, ou_all, l_all, s_scr, m_scr, zsm,
                   ksem, vsem, k0sem, wqsem, wsem, osem):
            wor_v, wo7_v, out_v = wqr_v, wq0_v, x_v

            def blk(t):
                if isinstance(t, int):
                    return t // 2, (t % 2) * P
                return lax.shift_right_logical(t, 1), (t & 1) * P

            def vcopy(t, slot):
                h, b0 = blk(t)
                return pltpu.make_async_copy(v_hbm.at[pl.ds(b0, P), h], vbuf.at[slot], vsem.at[slot])

            wocs = [pltpu.make_async_copy(wo_hbm.at[:, pl.ds(i * G * 128, G * 128)], wor_v.at[i], wsem.at[3])
                    for i in range(P)]
            wocs.append(pltpu.make_async_copy(wo_hbm.at[:, pl.ds(P * G * 128, W)], wo7_v, wsem.at[3]))

            xa = pltpu.make_async_copy(x_hbm.at[pl.ds(0, XR)], x_v.at[pl.ds(0, XR)], wsem.at[0])
            xb = pltpu.make_async_copy(x_hbm.at[pl.ds(XR, R - XR)], x_v.at[pl.ds(XR, R - XR)], wsem.at[1])
            wq0c = pltpu.make_async_copy(wq_hbm.at[:, pl.ds(0, W)], wq0_v, wsem.at[2])

            xa.start()
            wq0c.start()
            xb.start()

            def probs(i, ks):
                nt = (ks.stop - ks.start) // 128
                p = jnp.exp2(s_scr[i, :, ks] - jnp.concatenate([m_scr[i]] * nt, axis=1))
                l = p[:, 0:128]
                for c in range(1, nt):
                    l = l + p[:, c * 128:(c + 1) * 128]
                return p.astype(bf16), l

            def front(kbuf, q0, qs, qa, mr_scr, xB, wB):
                def kcopy(t, slot):
                    h, b0 = blk(t)
                    return pltpu.make_async_copy(k_hbm.at[pl.ds(b0, P), h], kbuf.at[slot], ksem.at[slot])

                def k0copy(i):
                    return pltpu.make_async_copy(k_hbm.at[i, 0], kbuf.at[0, i], k0sem.at[i])

                def wqrc(i):
                    return pltpu.make_async_copy(
                        wq_hbm.at[:, pl.ds(W + i * G * 128, G * 128)], wqr_v.at[i], wqsem.at[i])

                def qproj0(r0, r1):
                    q = jnp.dot(x_v[r0:r1, :], wq0_v[...], preferred_element_type=f32)
                    q = pltpu.bitcast((q * scale).astype(bf16), i32)
                    for b in range(r0 // Sq, r1 // Sq):
                        qb = q[(b * Sq - r0) // 2:((b + 1) * Sq - r0) // 2]
                        val = jnp.stack([qb[:, k * 128:(k + 1) * 128] for k in range(TPH)])
                        if b < P:
                            q0[b] = val
                        else:
                            qs[b - P] = val

                xa.wait()
                wq0c.wait()
                k0copy(0).start()
                wqrc(0).start()
                qproj0(0, XR)
                xb.wait()
                k0copy(1).start()
                wqrc(1).start()
                qproj0(XR, R)

                def load_q(ref, i):
                    q = ref[i]
                    return pltpu.bitcast(jnp.concatenate(
                        [jnp.concatenate([q[r * TPQ + c] for c in range(TPQ)], axis=1) for r in range(rep)],
                        axis=0), bf16)

                def colmax(s, mrun):
                    for c in range(s.shape[1] // 128):
                        sc = s[:, c * 128:(c + 1) * 128]
                        mrun = sc if mrun is None else jnp.maximum(mrun, sc)
                    return mrun

                def rowmax(mrun):
                    return jnp.broadcast_to(jnp.max(mrun, axis=-1, keepdims=True), (M, 128))

                def abody(i, zc):
                    k0copy(i).wait()
                    wqrc(i).wait()
                    zv = jnp.full((8, 128), zc[0] * zc[1], i32)
                    rg = R // arows

                    @pl.when(i + 2 < P)
                    def _():
                        wqrc(i + 2).start()

                    @pl.when(i + 2 < P)
                    def _():
                        k0copy(i + 2).start()

                    @pl.when(i == 0)
                    def _():
                        kcopy(1, 1).start()

                    @pl.when(i == 1)
                    def _():
                        vcopy(0, 0).start()

                    def qpart(g):
                        q = jnp.dot(x_v[g * rg:(g + 1) * rg, 0:DM], wqr_v[i, 0:DM, :], preferred_element_type=f32)
                        q = q * scale
                        qa[pl.ds(i * G, G), g * rg // 8:(g + 1) * rg // 8] = jnp.stack(
                            [q[:, k * 128:(k + 1) * 128].reshape(rg // 8, 8, 128) for k in range(G)])
                        return q

                    qp = qpart(0)
                    mrun = None
                    for k0 in range(0, Sk, KCE):
                        s = lax.dot_general(load_q(q0, i), kbuf[0, i, k0:k0 + KCE, :], NT,
                                            preferred_element_type=f32)
                        s_scr[i, :, k0:k0 + KCE] = s
                        mrun = colmax(s, mrun)
                    mx = rowmax(mrun)
                    m_scr[i] = mx
                    for g in range(1, arows):
                        qpart(g)

                    dep = _bits(mx[M - 8:M])
                    for u in range(2, M // 8 + 1):
                        dep = dep | _bits(mx[M - 8 * u:M - 8 * u + 8])
                    dep = jnp.concatenate([(dep & zv)[:, 0:KR]] * (TR // 16), axis=0)
                    xr = x_v[pl.ds(pl.multiple_of(i * TR, 16), TR), DM:D]
                    xr = pltpu.bitcast(pltpu.bitcast(xr, i32) | dep, bf16).astype(f32)
                    xB[:, pl.ds(i * (TR // 8), TR // 8)] = jnp.stack(
                        [jnp.broadcast_to(xr[:, kk:kk + 1], (TR, 128)).reshape(TR // 8, 8, 128) for kk in range(KR)])
                    wr = wqr_v[i, DM:D, :].astype(f32) * scale
                    nrg = rg // 8
                    wrows = []
                    for kk in range(KR):
                        n = kk * (nrg * G) // KR
                        dep = _bits(qp[(n % nrg) * 8:(n % nrg) * 8 + 8, (n // nrg) * 128:(n // nrg + 1) * 128]) & zv
                        wrow = jnp.broadcast_to(wr[kk:kk + 1, :], (8, G * 128))
                        wrows.append(_flt(_bits(wrow) | jnp.concatenate([dep] * G, axis=1)))
                    wall = jnp.stack(wrows)
                    wB[pl.ds(i * G, G)] = jnp.stack([wall[:, :, k * 128:(k + 1) * 128] for k in range(G)])
                    return (zc[1], zc[0])

                lax.fori_loop(0, P, abody, (jnp.int32(0), jnp.int32(1)))

                NC = Sk // KC
                RGS = [(i, r0) for i in range(P) for r0 in range(0, Sq, 16)]
                pieces = [RGS[n % len(RGS)] + ((n + n // len(RGS)) % TPH,) for n in range(len(RGS) * TPH)]
                assert len(set(pieces)) == len(pieces)
                due = [2 * NC * P * M - lead - (len(pieces) - 1 - n) * delta for n in range(len(pieces))]

                def body(t, slots):
                    sm1, s0 = slots
                    kcopy(t, s0).wait()
                    vcopy(t - 1, sm1).wait()
                    hp, bp0 = blk(t - 1)
                    hn, bn0 = blk(jnp.minimum(t + 1, NS - 1))
                    z1 = sm1 * s0
                    z2 = sm1 + s0 - 1
                    zvec = jnp.full((8, 128), z1, i32)
                    wt = [(hn - 1) * TPH + ct for ct in range(TPH)]
                    otile = pl.ds(hp * TPH, TPH)
                    ltile = pl.ds(hp * rep, rep)
                    rg0 = bn0 * (Sq // 8)
                    done = []
                    nmm = [0]

                    def piece():
                        i, r0, ct = pieces[len(done)]
                        rows = pl.ds(rg0 + (i * Sq + r0) // 8, 2)
                        acc = qa[wt[ct], rows][None]
                        for k0 in range(0, KR, gs):
                            xg = xB[k0:k0 + gs, rows]
                            wg = wB[wt[ct], k0:k0 + gs][:, None]
                            if k0 == pre and done:
                                acc = _flt(_bits(acc) | (done[-1] & zvec)[None, None])
                            prod = xg * wg
                            for u in range(gs):
                                acc = acc + prod[u:u + 1]
                        done.append(pltpu.bitcast(acc.reshape(16, 128).astype(bf16), i32))

                    def paced(val):
                        c = nmm[0]
                        nmm[0] += 1
                        while len(done) < len(pieces) and due[len(done)] < (c + 1) * M:
                            row = max(0, int(due[len(done)] - c * M)) // 8 * 8
                            piece()
                            val = _tie(val, row, done[-1] & zvec)
                        return val

                    for i in range(P):
                        rows = pl.ds(pl.multiple_of((bp0 + i) * Sq, 16), Sq)

                        def pv(j, pb, last):
                            o = jnp.dot(pb, vbuf[sm1, i, j * KC:(j + 1) * KC, :], preferred_element_type=f32)
                            if j > 0:
                                op = ou_all[otile, rows, :]
                                o = o + jnp.concatenate([jnp.concatenate(
                                    [op[r * TPQ + c] for c in range(TPQ)], axis=1) for r in range(rep)], axis=0)
                            vals = [o[:, c * 128:(c + 1) * 128] for c in range(TPQ)]
                            vals[0] = paced(vals[0])
                            if last:
                                res = dict(zip(pieces, done, strict=True))
                                step = M // 8 // ngrp * 8
                                per = len(RGS) // ngrp
                                for g in range(ngrp):
                                    vals[0] = _tie(vals[0], g * step, qs[z2, 0, 0:8, :] & zvec)
                                    grp = RGS[g * per:(g + 1) * per]
                                    pi, r0 = grp[0]
                                    assert grp[-1][0] == pi
                                    qs[pi + z1, :, r0 // 2:r0 // 2 + 8 * per, :] = jnp.stack(
                                        [jnp.concatenate([res[rg_ + (ct,)] for rg_ in grp], axis=0)
                                         for ct in range(TPH)])
                            ou_all[otile, rows, :] = jnp.stack(
                                [vals[c][r * Sq:(r + 1) * Sq] for r in range(rep) for c in range(TPQ)])

                        for j in range(NC):
                            ks = slice(j * KC, (j + 1) * KC)
                            last = i == P - 1 and j == NC - 1
                            pb, l = probs(i, ks)
                            l = l.reshape(rep, Sq, 128)
                            if j > 0:
                                l = l + l_all[ltile, rows, :]
                            l_all[ltile, rows, :] = l
                            if not last:
                                pv(j, pb, False)
                            if i == 0 and j == 0:
                                @pl.when(t + 1 < NS)
                                def _():
                                    kcopy(t + 1, sm1).start()

                                vcopy(t, s0).start()

                                @pl.when(t == NS - 2)
                                def _():
                                    for cc in wocs:
                                        cc.start()
                            s = lax.dot_general(load_q(qs, i), kbuf[s0, i, ks, :], NT, preferred_element_type=f32)
                            s_scr[i, :, ks] = jnp.concatenate([paced(s[:, 0:128]), s[:, 128:]], axis=1)
                            mrun = colmax(s, mr_scr[z1] if j > 0 else None)
                            if j < NC - 1:
                                mr_scr[z1] = mrun
                            else:
                                m_scr[i] = rowmax(mrun)
                            if last:
                                pv(j, pb, True)
                    return (s0, sm1)

                fin = lax.fori_loop(1, NS, body, (jnp.int32(0), jnp.int32(1)))
                zsm[0] = fin[0] * fin[1]

            def back(ou7, l7, accT, acc_n, on0):
                zero = zsm[0]

                def rows_of(big, small, idx_big, idx_small, r0, r1):
                    parts = []
                    if r0 < HR:
                        parts.append(big[idx_big, r0:min(r1, HR), :])
                    if r1 > HR:
                        parts.append(small[idx_small, max(r0, HR) - HR:r1 - HR, :])
                    return parts[0] if len(parts) == 1 else jnp.concatenate(parts, axis=0)

                def denom7(n):
                    r0, r1 = n * 128, (n + 1) * 128
                    return [jnp.broadcast_to(
                        jnp.sum(rows_of(l_all, l7, (Hkv - 1) * rep + r, r, r0, r1), axis=-1, keepdims=True), (128, 128))
                        for r in range(rep)]

                def normed7(n, ls):
                    r0, r1 = n * 128, (n + 1) * 128
                    tiles = []
                    for r in range(rep):
                        rc = _recip(ls[r])
                        for cc in range(TPQ):
                            k = r * TPQ + cc
                            tiles.append(rows_of(ou_all, ou7, (Hkv - 1) * TPH + k, k, r0, r1) * rc)
                    return jnp.concatenate(tiles, axis=1).astype(bf16)

                vlast = (NS - 1) % 2
                vcopy(NS - 1, vlast).wait()
                for cc in wocs:
                    cc.wait()

                def cbody(ii, c):
                    for u in range(CU):
                        i = ii * CU + u
                        rows = pl.ds(pl.multiple_of(i * Sq, 16), Sq)
                        o = None
                        l = None
                        for k0 in range(0, Sk, KCE):
                            pb, lj = probs(i, slice(k0, k0 + KCE))
                            l = lj if l is None else l + lj
                            if k0 + KCE == Sk:
                                l7[:, rows, :] = l.reshape(rep, Sq, 128)
                            oj = jnp.dot(pb, vbuf[vlast, i, k0:k0 + KCE, :], preferred_element_type=f32)
                            o = oj if o is None else oj + o
                        ou7[:, rows, :] = jnp.stack(
                            [o[r * Sq:(r + 1) * Sq, cc * 128:(cc + 1) * 128] for r in range(rep) for cc in range(TPQ)])
                    tiles = []
                    for k2 in range(CU * G // TPQ):
                        kq = ii * (CU * G // TPQ) + k2
                        rc = _recip(jnp.sum(l_all[kq], axis=-1, keepdims=True))
                        for cc in range(TPQ):
                            tiles.append(ou_all[kq * TPQ + cc] * rc)
                    on = jnp.concatenate(tiles, axis=1).astype(bf16)
                    w = jnp.concatenate([wor_v[ii * CU + u] for u in range(CU)], axis=1)
                    y = lax.dot_general(w, on, NT, preferred_element_type=f32) + jnp.where(ii > 0, accT[...], 0.0)
                    for n in range(npre):
                        on0[n] = pltpu.bitcast(normed7(n, denom7(n)), i32)
                    accT[...] = y
                    return c

                lax.fori_loop(0, P // CU, cbody, 0)

                dens = {n: denom7(n) for n in range(npre, NO)}
                dep = None
                for n in dens:
                    for l in dens[n]:
                        for u in range(16):
                            b = _bits(l[u * 8:u * 8 + 8])
                            dep = b if dep is None else dep | b
                dep = dep & jnp.full((8, 128), zero, i32)

                def after_sums(v):
                    for row in range(0, D, 128):
                        v = _tie(v, row, dep)
                    return v

                acc_n[...] = after_sums(accT[:, R - 128:R]).T
                ocs = []
                res = {}
                for n in range(NO + lag):
                    if n >= lag:
                        r0 = (n - lag) * 128
                        out_v[pl.ds(pl.multiple_of(r0 + zero, 128), 128), :] = res.pop(n - lag)
                        oc = pltpu.make_async_copy(
                            out_v.at[pl.ds(r0, 128)], out_hbm.at[pl.ds(r0, 128)], osem.at[n - lag])
                        oc.start()
                        ocs.append(oc)
                    if n >= NO:
                        continue
                    r0, r1 = n * 128, (n + 1) * 128
                    on = normed7(n, dens[n]) if n >= npre else pltpu.bitcast(on0[n], bf16)
                    if n >= lag:
                        rows = pl.ds(pl.multiple_of(r0 + zero, 128), 128)
                        out_v[rows, 0:128] = on[:, 0:128]
                        on = jnp.concatenate([out_v[rows, 0:128], on[:, 128:]], axis=1)
                    if n == NO - 1:
                        res[n] = (lax.dot_general(on, wo7_v[...], NT, preferred_element_type=f32)
                                  + acc_n[...]).astype(bf16)
                    else:
                        y = lax.dot_general(wo7_v[...], on, NT, preferred_element_type=f32) + accT[:, r0:r1]
                        res[n] = (after_sums(y) if n < 2 else y).astype(bf16).T
                for oc in ocs:
                    oc.wait()

            def stage(u, c):
                @pl.when(u == 0)
                def _():
                    pl.run_scoped(
                        front,
                        pltpu.VMEM((2, P, Sk, Dh), bf16),
                        pltpu.VMEM((P, TPH, Sq // 2, 128), i32),
                        pltpu.VMEM((P, TPH, Sq // 2, 128), i32),
                        pltpu.VMEM((NTL - TPH, R // 8, 8, 128), f32),
                        pltpu.VMEM((2, M, 128), f32),
                        pltpu.VMEM((KR, R // 8 + 1, 8, 128), f32),
                        pltpu.VMEM((NTL - TPH, KR, 8, 128), f32),
                    )

                @pl.when(u == 1)
                def _():
                    pl.run_scoped(
                        back,
                        pltpu.VMEM((TPH, HR, 128), f32),
                        pltpu.VMEM((rep, HR, 128), f32),
                        pltpu.VMEM((D, R), f32),
                        pltpu.VMEM((128, D), f32),
                        pltpu.VMEM((npre, 64, W), i32),
                    )
                return c

            lax.fori_loop(0, 2, stage, 0)

        out = pl.pallas_call(
            kernel,
            in_specs=[pl.BlockSpec(memory_space=pl.ANY)] * 5,
            out_specs=pl.BlockSpec(memory_space=pl.ANY),
            out_shape=jax.ShapeDtypeStruct((R, D), x.dtype),
            scratch_shapes=[
                pltpu.VMEM((R, D), bf16),
                pltpu.VMEM((D, W), bf16),
                pltpu.VMEM((P, D, G * 128), bf16),
                pltpu.VMEM((2, P, Sk, Dh), bf16),
                pltpu.VMEM((NTL, R, 128), f32),
                pltpu.VMEM((Hq, R, 128), f32),
                pltpu.VMEM((P, M, Sk), f32),
                pltpu.VMEM((P, M, 128), f32),
                pltpu.SMEM((1,), i32),
                pltpu.SemaphoreType.DMA((2,)),
                pltpu.SemaphoreType.DMA((2,)),
                pltpu.SemaphoreType.DMA((P,)),
                pltpu.SemaphoreType.DMA((P,)),
                pltpu.SemaphoreType.DMA((4,)),
                pltpu.SemaphoreType.DMA((NO,)),
            ],
            compiler_params=pltpu.CompilerParams(
                vmem_limit_bytes=vmem * 1024 * 1024,
                disable_bounds_checks=not checks,
                disable_semaphore_checks=not checks,
            ),
        )(x.reshape(R, D), k_cache, v_cache, wq, wo.T)
        return out.reshape(B, Sq, D)
    return fn


@jax.jit
def pallas_standalone__gqa_block_cached__near_ridge_kernel(
    x: jax.Array,
    k_cache: jax.Array,
    v_cache: jax.Array,
    wq: jax.Array,
    wo: jax.Array,
):
    return _make()(x, k_cache, v_cache, wq, wo)
```

```python
import jax
import jax.numpy as jnp
from jax import lax
import jax.experimental.pallas as pl
import jax.experimental.pallas.tpu as pltpu

LOG2E = 1.4426950408889634
f32, bf16, i32 = jnp.float32, jnp.bfloat16, jnp.int32
NT = (((1,), (1,)), ((), ()))


def _bits(v):
    return lax.bitcast_convert_type(v, i32)


def _flt(v):
    return lax.bitcast_convert_type(v, f32)


def _recip(l):
    r = pl.reciprocal(l, approx=True)
    return r * (2.0 - l * r)


def _tie(val, row, dep):
    parts = [val[:row]] if row else []
    parts.append(_flt(_bits(val[row:row + 8]) | dep))
    if row + 8 < val.shape[0]:
        parts.append(val[row + 8:])
    return jnp.concatenate(parts, axis=0)


def _make(KC=256, KCE=512, vmem=127, checks=False, xsplit=2, CU=2, arows=4, lag=2,
         pre=8, ngrp=12, gs=8, lead=42, delta=125.32, npre=4):
    P = 4

    def fn(x, k_cache, v_cache, wq, wo):
        B, Sq, D = x.shape
        _, Hkv, Sk, Dh = k_cache.shape
        Hq = wq.shape[1] // Dh
        rep = Hq // Hkv
        M = rep * Sq
        W = rep * Dh
        R = B * Sq
        TPH = W // 128
        TPQ = Dh // 128
        NTL = Hq * Dh // 128
        G = (NTL - TPH) // P
        DM = (D // 128) * 128
        KR = D - DM
        NS = B * Hkv // P
        HR = P * Sq
        NO = R // 128
        XR = xsplit * Sq
        TR = R // P
        assert G * P == NTL - TPH and B == 2 * P and R % 128 == 0 and Sq % 16 == 0 and TR % 16 == 0
        assert KR % gs == 0 and pre % gs == 0 and (CU * G) % TPQ == 0
        scale = Dh ** -0.5 * LOG2E

        def kernel(x_hbm, k_hbm, v_hbm, wq_hbm, wo_hbm, out_hbm,
                   x_v, wq0_v, wqr_v, vbuf, ou_all, l_all, s_scr, m_scr, zsm,
                   ksem, vsem, k0sem, wqsem, wsem, osem):
            wor_v, wo7_v, out_v = wqr_v, wq0_v, x_v

            def blk(t):
                if isinstance(t, int):
                    return t // 2, (t % 2) * P
                return lax.shift_right_logical(t, 1), (t & 1) * P

            def vcopy(t, slot):
                h, b0 = blk(t)
                return pltpu.make_async_copy(v_hbm.at[pl.ds(b0, P), h], vbuf.at[slot], vsem.at[slot])

            wocs = [pltpu.make_async_copy(wo_hbm.at[:, pl.ds(i * G * 128, G * 128)], wor_v.at[i], wsem.at[3])
                    for i in range(P)]
            wocs.append(pltpu.make_async_copy(wo_hbm.at[:, pl.ds(P * G * 128, W)], wo7_v, wsem.at[3]))

            xa = pltpu.make_async_copy(x_hbm.at[pl.ds(0, XR)], x_v.at[pl.ds(0, XR)], wsem.at[0])
            xb = pltpu.make_async_copy(x_hbm.at[pl.ds(XR, R - XR)], x_v.at[pl.ds(XR, R - XR)], wsem.at[1])
            wq0c = pltpu.make_async_copy(wq_hbm.at[:, pl.ds(0, W)], wq0_v, wsem.at[2])

            xa.start()
            wq0c.start()
            xb.start()

            def probs(i, ks):
                nt = (ks.stop - ks.start) // 128
                p = jnp.exp2(s_scr[i, :, ks] - jnp.concatenate([m_scr[i]] * nt, axis=1))
                l = p[:, 0:128]
                for c in range(1, nt):
                    l = l + p[:, c * 128:(c + 1) * 128]
                return p.astype(bf16), l

            def front(kbuf, q0, qs, qa, mr_scr, xB, wB):
                def kcopy(t, slot):
                    h, b0 = blk(t)
                    return pltpu.make_async_copy(k_hbm.at[pl.ds(b0, P), h], kbuf.at[slot], ksem.at[slot])

                def k0copy(i):
                    return pltpu.make_async_copy(k_hbm.at[i, 0], kbuf.at[0, i], k0sem.at[i])

                def wqrc(i):
                    return pltpu.make_async_copy(
                        wq_hbm.at[:, pl.ds(W + i * G * 128, G * 128)], wqr_v.at[i], wqsem.at[i])

                def qproj0(r0, r1):
                    q = jnp.dot(x_v[r0:r1, :], wq0_v[...], preferred_element_type=f32)
                    q = pltpu.bitcast((q * scale).astype(bf16), i32)
                    for b in range(r0 // Sq, r1 // Sq):
                        qb = q[(b * Sq - r0) // 2:((b + 1) * Sq - r0) // 2]
                        val = jnp.stack([qb[:, k * 128:(k + 1) * 128] for k in range(TPH)])
                        if b < P:
                            q0[b] = val
                        else:
                            qs[b - P] = val

                xa.wait()
                wq0c.wait()
                k0copy(0).start()
                wqrc(0).start()
                qproj0(0, XR)
                xb.wait()
                k0copy(1).start()
                wqrc(1).start()
                qproj0(XR, R)

                def load_q(ref, i):
                    q = ref[i]
                    return pltpu.bitcast(jnp.concatenate(
                        [jnp.concatenate([q[r * TPQ + c] for c in range(TPQ)], axis=1) for r in range(rep)],
                        axis=0), bf16)

                def colmax(s, mrun):
                    for c in range(s.shape[1] // 128):
                        sc = s[:, c * 128:(c + 1) * 128]
                        mrun = sc if mrun is None else jnp.maximum(mrun, sc)
                    return mrun

                def rowmax(mrun):
                    return jnp.broadcast_to(jnp.max(mrun, axis=-1, keepdims=True), (M, 128))

                def abody(i, zc):
                    k0copy(i).wait()
                    wqrc(i).wait()
                    zv = jnp.full((8, 128), zc[0] * zc[1], i32)
                    rg = R // arows

                    @pl.when(i + 2 < P)
                    def _():
                        wqrc(i + 2).start()

                    @pl.when(i + 2 < P)
                    def _():
                        k0copy(i + 2).start()

                    @pl.when(i == 0)
                    def _():
                        kcopy(1, 1).start()

                    @pl.when(i == 1)
                    def _():
                        vcopy(0, 0).start()

                    def qpart(g):
                        q = jnp.dot(x_v[g * rg:(g + 1) * rg, 0:DM], wqr_v[i, 0:DM, :], preferred_element_type=f32)
                        q = q * scale
                        qa[pl.ds(i * G, G), g * rg // 8:(g + 1) * rg // 8] = jnp.stack(
                            [q[:, k * 128:(k + 1) * 128].reshape(rg // 8, 8, 128) for k in range(G)])
                        return q

                    qp = qpart(0)
                    mrun = None
                    for k0 in range(0, Sk, KCE):
                        s = lax.dot_general(load_q(q0, i), kbuf[0, i, k0:k0 + KCE, :], NT,
                                            preferred_element_type=f32)
                        s_scr[i, :, k0:k0 + KCE] = s
                        mrun = colmax(s, mrun)
                    mx = rowmax(mrun)
                    m_scr[i] = mx
                    for g in range(1, arows):
                        qpart(g)

                    dep = _bits(mx[M - 8:M])
                    for u in range(2, M // 8 + 1):
                        dep = dep | _bits(mx[M - 8 * u:M - 8 * u + 8])
                    dep = jnp.concatenate([(dep & zv)[:, 0:KR]] * (TR // 16), axis=0)
                    xr = x_v[pl.ds(pl.multiple_of(i * TR, 16), TR), DM:D]
                    xr = pltpu.bitcast(pltpu.bitcast(xr, i32) | dep, bf16).astype(f32)
                    xB[:, pl.ds(i * (TR // 8), TR // 8)] = jnp.stack(
                        [jnp.broadcast_to(xr[:, kk:kk + 1], (TR, 128)).reshape(TR // 8, 8, 128) for kk in range(KR)])
                    wr = wqr_v[i, DM:D, :].astype(f32) * scale
                    nrg = rg // 8
                    wrows = []
                    for kk in range(KR):
                        n = kk * (nrg * G) // KR
                        dep = _bits(qp[(n % nrg) * 8:(n % nrg) * 8 + 8, (n // nrg) * 128:(n // nrg + 1) * 128]) & zv
                        wrow = jnp.broadcast_to(wr[kk:kk + 1, :], (8, G * 128))
                        wrows.append(_flt(_bits(wrow) | jnp.concatenate([dep] * G, axis=1)))
                    wall = jnp.stack(wrows)
                    wB[pl.ds(i * G, G)] = jnp.stack([wall[:, :, k * 128:(k + 1) * 128] for k in range(G)])
                    return (zc[1], zc[0])

                lax.fori_loop(0, P, abody, (jnp.int32(0), jnp.int32(1)))

                NC = Sk // KC
                RGS = [(i, r0) for i in range(P) for r0 in range(0, Sq, 16)]
                pieces = [RGS[n % len(RGS)] + ((n + n // len(RGS)) % TPH,) for n in range(len(RGS) * TPH)]
                assert len(set(pieces)) == len(pieces)
                due = [2 * NC * P * M - lead - (len(pieces) - 1 - n) * delta for n in range(len(pieces))]

                def body(t, slots):
                    sm1, s0 = slots
                    kcopy(t, s0).wait()
                    vcopy(t - 1, sm1).wait()
                    hp, bp0 = blk(t - 1)
                    hn, bn0 = blk(jnp.minimum(t + 1, NS - 1))
                    z1 = sm1 * s0
                    z2 = sm1 + s0 - 1
                    zvec = jnp.full((8, 128), z1, i32)
                    wt = [(hn - 1) * TPH + ct for ct in range(TPH)]
                    otile = pl.ds(hp * TPH, TPH)
                    ltile = pl.ds(hp * rep, rep)
                    rg0 = bn0 * (Sq // 8)
                    done = []
                    nmm = [0]

                    def piece():
                        i, r0, ct = pieces[len(done)]
                        rows = pl.ds(rg0 + (i * Sq + r0) // 8, 2)
                        acc = qa[wt[ct], rows][None]
                        for k0 in range(0, KR, gs):
                            xg = xB[k0:k0 + gs, rows]
                            wg = wB[wt[ct], k0:k0 + gs][:, None]
                            if k0 == pre and done:
                                acc = _flt(_bits(acc) | (done[-1] & zvec)[None, None])
                            acc = jnp.sum(jnp.concatenate([acc, xg * wg], axis=0), axis=0, keepdims=True)
                        done.append(pltpu.bitcast(acc.reshape(16, 128).astype(bf16), i32))

                    def paced(val):
                        c = nmm[0]
                        nmm[0] += 1
                        while len(done) < len(pieces) and due[len(done)] < (c + 1) * M:
                            row = max(0, int(due[len(done)] - c * M)) // 8 * 8
                            piece()
                            val = _tie(val, row, done[-1] & zvec)
                        return val

                    for i in range(P):
                        rows = pl.ds(pl.multiple_of((bp0 + i) * Sq, 16), Sq)

                        def pv(j, pb, last):
                            o = jnp.dot(pb, vbuf[sm1, i, j * KC:(j + 1) * KC, :], preferred_element_type=f32)
                            if j > 0:
                                op = ou_all[otile, rows, :]
                                o = o + jnp.concatenate([jnp.concatenate(
                                    [op[r * TPQ + c] for c in range(TPQ)], axis=1) for r in range(rep)], axis=0)
                            vals = [o[:, c * 128:(c + 1) * 128] for c in range(TPQ)]
                            vals[0] = paced(vals[0])
                            if last:
                                res = dict(zip(pieces, done, strict=True))
                                step = M // 8 // ngrp * 8
                                per = len(RGS) // ngrp
                                for g in range(ngrp):
                                    vals[0] = _tie(vals[0], g * step, qs[z2, 0, 0:8, :] & zvec)
                                    grp = RGS[g * per:(g + 1) * per]
                                    pi, r0 = grp[0]
                                    assert grp[-1][0] == pi
                                    qs[pi + z1, :, r0 // 2:r0 // 2 + 8 * per, :] = jnp.stack(
                                        [jnp.concatenate([res[rg_ + (ct,)] for rg_ in grp], axis=0)
                                         for ct in range(TPH)])
                            ou_all[otile, rows, :] = jnp.stack(
                                [vals[c][r * Sq:(r + 1) * Sq] for r in range(rep) for c in range(TPQ)])

                        for j in range(NC):
                            ks = slice(j * KC, (j + 1) * KC)
                            last = i == P - 1 and j == NC - 1
                            pb, l = probs(i, ks)
                            l = l.reshape(rep, Sq, 128)
                            if j > 0:
                                l = l + l_all[ltile, rows, :]
                            l_all[ltile, rows, :] = l
                            if not last:
                                pv(j, pb, False)
                            if i == 0 and j == 0:
                                @pl.when(t + 1 < NS)
                                def _():
                                    kcopy(t + 1, sm1).start()

                                vcopy(t, s0).start()

                                @pl.when(t == NS - 2)
                                def _():
                                    for cc in wocs:
                                        cc.start()
                            s = lax.dot_general(load_q(qs, i), kbuf[s0, i, ks, :], NT, preferred_element_type=f32)
                            s_scr[i, :, ks] = jnp.concatenate([paced(s[:, 0:128]), s[:, 128:]], axis=1)
                            mrun = colmax(s, mr_scr[z1] if j > 0 else None)
                            if j < NC - 1:
                                mr_scr[z1] = mrun
                            else:
                                m_scr[i] = rowmax(mrun)
                            if last:
                                pv(j, pb, True)
                    return (s0, sm1)

                fin = lax.fori_loop(1, NS, body, (jnp.int32(0), jnp.int32(1)))
                zsm[0] = fin[0] * fin[1]

            def back(ou7, l7, accT, acc_n, on0):
                zero = zsm[0]

                def rows_of(big, small, idx_big, idx_small, r0, r1):
                    parts = []
                    if r0 < HR:
                        parts.append(big[idx_big, r0:min(r1, HR), :])
                    if r1 > HR:
                        parts.append(small[idx_small, max(r0, HR) - HR:r1 - HR, :])
                    return parts[0] if len(parts) == 1 else jnp.concatenate(parts, axis=0)

                def denom7(n):
                    r0, r1 = n * 128, (n + 1) * 128
                    return [jnp.broadcast_to(
                        jnp.sum(rows_of(l_all, l7, (Hkv - 1) * rep + r, r, r0, r1), axis=-1, keepdims=True), (128, 128))
                        for r in range(rep)]

                def normed7(n, ls):
                    r0, r1 = n * 128, (n + 1) * 128
                    tiles = []
                    for r in range(rep):
                        rc = _recip(ls[r])
                        for cc in range(TPQ):
                            k = r * TPQ + cc
                            tiles.append(rows_of(ou_all, ou7, (Hkv - 1) * TPH + k, k, r0, r1) * rc)
                    return jnp.concatenate(tiles, axis=1).astype(bf16)

                vlast = (NS - 1) % 2
                vcopy(NS - 1, vlast).wait()
                for cc in wocs:
                    cc.wait()

                def cbody(ii, c):
                    for u in range(CU):
                        i = ii * CU + u
                        rows = pl.ds(pl.multiple_of(i * Sq, 16), Sq)
                        o = None
                        l = None
                        for k0 in range(0, Sk, KCE):
                            pb, lj = probs(i, slice(k0, k0 + KCE))
                            l = lj if l is None else l + lj
                            if k0 + KCE == Sk:
                                l7[:, rows, :] = l.reshape(rep, Sq, 128)
                            oj = jnp.dot(pb, vbuf[vlast, i, k0:k0 + KCE, :], preferred_element_type=f32)
                            o = oj if o is None else oj + o
                        ou7[:, rows, :] = jnp.stack(
                            [o[r * Sq:(r + 1) * Sq, cc * 128:(cc + 1) * 128] for r in range(rep) for cc in range(TPQ)])
                    tiles = []
                    for k2 in range(CU * G // TPQ):
                        kq = ii * (CU * G // TPQ) + k2
                        rc = _recip(jnp.sum(l_all[kq], axis=-1, keepdims=True))
                        for cc in range(TPQ):
                            tiles.append(ou_all[kq * TPQ + cc] * rc)
                    on = jnp.concatenate(tiles, axis=1).astype(bf16)
                    w = jnp.concatenate([wor_v[ii * CU + u] for u in range(CU)], axis=1)
                    y = lax.dot_general(w, on, NT, preferred_element_type=f32) + jnp.where(ii > 0, accT[...], 0.0)
                    for n in range(npre):
                        on0[n] = pltpu.bitcast(normed7(n, denom7(n)), i32)
                    accT[...] = y
                    return c

                lax.fori_loop(0, P // CU, cbody, 0)

                dens = {n: denom7(n) for n in range(npre, NO)}
                dep = None
                for n in dens:
                    for l in dens[n]:
                        for u in range(16):
                            b = _bits(l[u * 8:u * 8 + 8])
                            dep = b if dep is None else dep | b
                dep = dep & jnp.full((8, 128), zero, i32)

                def after_sums(v):
                    for row in range(0, D, 128):
                        v = _tie(v, row, dep)
                    return v

                acc_n[...] = after_sums(accT[:, R - 128:R]).T
                ocs = []
                res = {}
                for n in range(NO + lag):
                    if n >= lag:
                        r0 = (n - lag) * 128
                        out_v[pl.ds(pl.multiple_of(r0 + zero, 128), 128), :] = res.pop(n - lag)
                        oc = pltpu.make_async_copy(
                            out_v.at[pl.ds(r0, 128)], out_hbm.at[pl.ds(r0, 128)], osem.at[n - lag])
                        oc.start()
                        ocs.append(oc)
                    if n >= NO:
                        continue
                    r0, r1 = n * 128, (n + 1) * 128
                    on = normed7(n, dens[n]) if n >= npre else pltpu.bitcast(on0[n], bf16)
                    if n >= lag:
                        rows = pl.ds(pl.multiple_of(r0 + zero, 128), 128)
                        out_v[rows, 0:128] = on[:, 0:128]
                        on = jnp.concatenate([out_v[rows, 0:128], on[:, 128:]], axis=1)
                    if n == NO - 1:
                        res[n] = (lax.dot_general(on, wo7_v[...], NT, preferred_element_type=f32)
                                  + acc_n[...]).astype(bf16)
                    else:
                        y = lax.dot_general(wo7_v[...], on, NT, preferred_element_type=f32) + accT[:, r0:r1]
                        res[n] = (after_sums(y) if n < 2 else y).astype(bf16).T
                for oc in ocs:
                    oc.wait()

            def stage(u, c):
                @pl.when(u == 0)
                def _():
                    pl.run_scoped(
                        front,
                        pltpu.VMEM((2, P, Sk, Dh), bf16),
                        pltpu.VMEM((P, TPH, Sq // 2, 128), i32),
                        pltpu.VMEM((P, TPH, Sq // 2, 128), i32),
                        pltpu.VMEM((NTL - TPH, R // 8, 8, 128), f32),
                        pltpu.VMEM((2, M, 128), f32),
                        pltpu.VMEM((KR, R // 8 + 1, 8, 128), f32),
                        pltpu.VMEM((NTL - TPH, KR, 8, 128), f32),
                    )

                @pl.when(u == 1)
                def _():
                    pl.run_scoped(
                        back,
                        pltpu.VMEM((TPH, HR, 128), f32),
                        pltpu.VMEM((rep, HR, 128), f32),
                        pltpu.VMEM((D, R), f32),
                        pltpu.VMEM((128, D), f32),
                        pltpu.VMEM((npre, 64, W), i32),
                    )
                return c

            lax.fori_loop(0, 2, stage, 0)

        out = pl.pallas_call(
            kernel,
            in_specs=[pl.BlockSpec(memory_space=pl.ANY)] * 5,
            out_specs=pl.BlockSpec(memory_space=pl.ANY),
            out_shape=jax.ShapeDtypeStruct((R, D), x.dtype),
            scratch_shapes=[
                pltpu.VMEM((R, D), bf16),
                pltpu.VMEM((D, W), bf16),
                pltpu.VMEM((P, D, G * 128), bf16),
                pltpu.VMEM((2, P, Sk, Dh), bf16),
                pltpu.VMEM((NTL, R, 128), f32),
                pltpu.VMEM((Hq, R, 128), f32),
                pltpu.VMEM((P, M, Sk), f32),
                pltpu.VMEM((P, M, 128), f32),
                pltpu.SMEM((1,), i32),
                pltpu.SemaphoreType.DMA((2,)),
                pltpu.SemaphoreType.DMA((2,)),
                pltpu.SemaphoreType.DMA((P,)),
                pltpu.SemaphoreType.DMA((P,)),
                pltpu.SemaphoreType.DMA((4,)),
                pltpu.SemaphoreType.DMA((NO,)),
            ],
            compiler_params=pltpu.CompilerParams(
                vmem_limit_bytes=vmem * 1024 * 1024,
                disable_bounds_checks=not checks,
                disable_semaphore_checks=not checks,
            ),
        )(x.reshape(R, D), k_cache, v_cache, wq, wo.T)
        return out.reshape(B, Sq, D)
    return fn


@jax.jit
def pallas_standalone__gqa_block_cached__near_ridge_kernel(
    x: jax.Array,
    k_cache: jax.Array,
    v_cache: jax.Array,
    wq: jax.Array,
    wo: jax.Array,
):
    return _make()(x, k_cache, v_cache, wq, wo)
```

```python
import jax
import jax.numpy as jnp
from jax import lax
import jax.experimental.pallas as pl
import jax.experimental.pallas.tpu as pltpu

LOG2E = 1.4426950408889634
f32, bf16, i32 = jnp.float32, jnp.bfloat16, jnp.int32
NT = (((1,), (1,)), ((), ()))


def _bits(v):
    return lax.bitcast_convert_type(v, i32)


def _flt(v):
    return lax.bitcast_convert_type(v, f32)


def _recip(l):
    r = pl.reciprocal(l, approx=True)
    return r * (2.0 - l * r)


def _tie(val, row, dep):
    parts = [val[:row]] if row else []
    parts.append(_flt(_bits(val[row:row + 8]) | dep))
    if row + 8 < val.shape[0]:
        parts.append(val[row + 8:])
    return jnp.concatenate(parts, axis=0)


P = 4
KC = 256
KCE = 512
XSPLIT = 2
CU = 2
AROWS = 4
LAG = 2
NPRE = 4
GS = 8
PRE = 8
LEAD = 42
DELTA = 125.32
NGRP = 12


@jax.jit
def pallas_standalone__gqa_block_cached__near_ridge_kernel(
    x: jax.Array,
    k_cache: jax.Array,
    v_cache: jax.Array,
    wq: jax.Array,
    wo: jax.Array,
):
    B, Sq, D = x.shape
    _, Hkv, Sk, Dh = k_cache.shape
    Hq = wq.shape[1] // Dh
    rep = Hq // Hkv
    M = rep * Sq
    W = rep * Dh
    R = B * Sq
    TPH = W // 128
    TPQ = Dh // 128
    NTL = Hq * Dh // 128
    G = (NTL - TPH) // P
    DM = (D // 128) * 128
    KR = D - DM
    NS = B * Hkv // P
    HR = P * Sq
    NO = R // 128
    XR = XSPLIT * Sq
    TR = R // P
    assert G * P == NTL - TPH and B == 2 * P and R % 128 == 0 and Sq % 16 == 0 and TR % 16 == 0
    assert KR % GS == 0 and PRE % GS == 0 and (CU * G) % TPQ == 0
    scale = Dh ** -0.5 * LOG2E

    def kernel(x_hbm, k_hbm, v_hbm, wq_hbm, wo_hbm, out_hbm,
               x_v, wq0_v, wqr_v, vbuf, ou_all, l_all, s_scr, m_scr, zsm,
               ksem, vsem, k0sem, wqsem, wsem, osem):
        wor_v, wo7_v, out_v = wqr_v, wq0_v, x_v

        def blk(t):
            if isinstance(t, int):
                return t // 2, (t % 2) * P
            return lax.shift_right_logical(t, 1), (t & 1) * P

        def vcopy(t, slot):
            h, b0 = blk(t)
            return pltpu.make_async_copy(v_hbm.at[pl.ds(b0, P), h], vbuf.at[slot], vsem.at[slot])

        wocs = [pltpu.make_async_copy(wo_hbm.at[:, pl.ds(i * G * 128, G * 128)], wor_v.at[i], wsem.at[3])
                for i in range(P)]
        wocs.append(pltpu.make_async_copy(wo_hbm.at[:, pl.ds(P * G * 128, W)], wo7_v, wsem.at[3]))

        xa = pltpu.make_async_copy(x_hbm.at[pl.ds(0, XR)], x_v.at[pl.ds(0, XR)], wsem.at[0])
        xb = pltpu.make_async_copy(x_hbm.at[pl.ds(XR, R - XR)], x_v.at[pl.ds(XR, R - XR)], wsem.at[1])
        wq0c = pltpu.make_async_copy(wq_hbm.at[:, pl.ds(0, W)], wq0_v, wsem.at[2])

        xa.start()
        wq0c.start()
        xb.start()

        def probs(i, ks):
            nt = (ks.stop - ks.start) // 128
            p = jnp.exp2(s_scr[i, :, ks] - jnp.concatenate([m_scr[i]] * nt, axis=1))
            l = p[:, 0:128]
            for c in range(1, nt):
                l = l + p[:, c * 128:(c + 1) * 128]
            return p.astype(bf16), l

        def front(kbuf, q0, qs, qa, mr_scr, xB, wB):
            def kcopy(t, slot):
                h, b0 = blk(t)
                return pltpu.make_async_copy(k_hbm.at[pl.ds(b0, P), h], kbuf.at[slot], ksem.at[slot])

            def k0copy(i):
                return pltpu.make_async_copy(k_hbm.at[i, 0], kbuf.at[0, i], k0sem.at[i])

            def wqrc(i):
                return pltpu.make_async_copy(
                    wq_hbm.at[:, pl.ds(W + i * G * 128, G * 128)], wqr_v.at[i], wqsem.at[i])

            def qproj0(r0, r1):
                q = jnp.dot(x_v[r0:r1, :], wq0_v[...], preferred_element_type=f32)
                q = pltpu.bitcast((q * scale).astype(bf16), i32)
                for b in range(r0 // Sq, r1 // Sq):
                    qb = q[(b * Sq - r0) // 2:((b + 1) * Sq - r0) // 2]
                    val = jnp.stack([qb[:, k * 128:(k + 1) * 128] for k in range(TPH)])
                    if b < P:
                        q0[b] = val
                    else:
                        qs[b - P] = val

            xa.wait()
            wq0c.wait()
            k0copy(0).start()
            wqrc(0).start()
            qproj0(0, XR)
            xb.wait()
            k0copy(1).start()
            wqrc(1).start()
            qproj0(XR, R)

            def load_q(ref, i):
                q = ref[i]
                return pltpu.bitcast(jnp.concatenate(
                    [jnp.concatenate([q[r * TPQ + c] for c in range(TPQ)], axis=1) for r in range(rep)],
                    axis=0), bf16)

            def colmax(s, mrun):
                for c in range(s.shape[1] // 128):
                    sc = s[:, c * 128:(c + 1) * 128]
                    mrun = sc if mrun is None else jnp.maximum(mrun, sc)
                return mrun

            def rowmax(mrun):
                return jnp.broadcast_to(jnp.max(mrun, axis=-1, keepdims=True), (M, 128))

            def abody(i, zc):
                k0copy(i).wait()
                wqrc(i).wait()
                zv = jnp.full((8, 128), zc[0] * zc[1], i32)
                rg = R // AROWS

                @pl.when(i + 2 < P)
                def _():
                    wqrc(i + 2).start()

                @pl.when(i + 2 < P)
                def _():
                    k0copy(i + 2).start()

                @pl.when(i == 0)
                def _():
                    kcopy(1, 1).start()

                @pl.when(i == 1)
                def _():
                    vcopy(0, 0).start()

                def qpart(g):
                    q = jnp.dot(x_v[g * rg:(g + 1) * rg, 0:DM], wqr_v[i, 0:DM, :], preferred_element_type=f32)
                    q = q * scale
                    qa[pl.ds(i * G, G), g * rg // 8:(g + 1) * rg // 8] = jnp.stack(
                        [q[:, k * 128:(k + 1) * 128].reshape(rg // 8, 8, 128) for k in range(G)])
                    return q

                qp = qpart(0)
                mrun = None
                for k0 in range(0, Sk, KCE):
                    s = lax.dot_general(load_q(q0, i), kbuf[0, i, k0:k0 + KCE, :], NT,
                                        preferred_element_type=f32)
                    s_scr[i, :, k0:k0 + KCE] = s
                    mrun = colmax(s, mrun)
                mx = rowmax(mrun)
                m_scr[i] = mx
                for g in range(1, AROWS):
                    qpart(g)

                dep = _bits(mx[M - 8:M])
                for u in range(2, M // 8 + 1):
                    dep = dep | _bits(mx[M - 8 * u:M - 8 * u + 8])
                dep = jnp.concatenate([(dep & zv)[:, 0:KR]] * (TR // 16), axis=0)
                xr = x_v[pl.ds(pl.multiple_of(i * TR, 16), TR), DM:D]
                xr = pltpu.bitcast(pltpu.bitcast(xr, i32) | dep, bf16).astype(f32)
                xB[:, pl.ds(i * (TR // 8), TR // 8)] = jnp.stack(
                    [jnp.broadcast_to(xr[:, kk:kk + 1], (TR, 128)).reshape(TR // 8, 8, 128) for kk in range(KR)])
                wr = wqr_v[i, DM:D, :].astype(f32) * scale
                nrg = rg // 8
                wrows = []
                for kk in range(KR):
                    n = kk * (nrg * G) // KR
                    dep = _bits(qp[(n % nrg) * 8:(n % nrg) * 8 + 8, (n // nrg) * 128:(n // nrg + 1) * 128]) & zv
                    wrow = jnp.broadcast_to(wr[kk:kk + 1, :], (8, G * 128))
                    wrows.append(_flt(_bits(wrow) | jnp.concatenate([dep] * G, axis=1)))
                wall = jnp.stack(wrows)
                wB[pl.ds(i * G, G)] = jnp.stack([wall[:, :, k * 128:(k + 1) * 128] for k in range(G)])
                return (zc[1], zc[0])

            lax.fori_loop(0, P, abody, (jnp.int32(0), jnp.int32(1)))

            NC = Sk // KC
            RGS = [(i, r0) for i in range(P) for r0 in range(0, Sq, 16)]
            pieces = [RGS[n % len(RGS)] + ((n + n // len(RGS)) % TPH,) for n in range(len(RGS) * TPH)]
            assert len(set(pieces)) == len(pieces)
            due = [2 * NC * P * M - LEAD - (len(pieces) - 1 - n) * DELTA for n in range(len(pieces))]

            def body(t, slots):
                sm1, s0 = slots
                kcopy(t, s0).wait()
                vcopy(t - 1, sm1).wait()
                hp, bp0 = blk(t - 1)
                hn, bn0 = blk(jnp.minimum(t + 1, NS - 1))
                z1 = sm1 * s0
                z2 = sm1 + s0 - 1
                zvec = jnp.full((8, 128), z1, i32)
                wt = [(hn - 1) * TPH + ct for ct in range(TPH)]
                otile = pl.ds(hp * TPH, TPH)
                ltile = pl.ds(hp * rep, rep)
                rg0 = bn0 * (Sq // 8)
                done = []
                nmm = [0]

                def piece():
                    i, r0, ct = pieces[len(done)]
                    rows = pl.ds(rg0 + (i * Sq + r0) // 8, 2)
                    acc = qa[wt[ct], rows][None]
                    for k0 in range(0, KR, GS):
                        xg = xB[k0:k0 + GS, rows]
                        wg = wB[wt[ct], k0:k0 + GS][:, None]
                        if k0 == PRE and done:
                            acc = _flt(_bits(acc) | (done[-1] & zvec)[None, None])
                        acc = jnp.sum(jnp.concatenate([acc, xg * wg], axis=0), axis=0, keepdims=True)
                    done.append(pltpu.bitcast(acc.reshape(16, 128).astype(bf16), i32))

                def paced(val):
                    c = nmm[0]
                    nmm[0] += 1
                    while len(done) < len(pieces) and due[len(done)] < (c + 1) * M:
                        row = max(0, int(due[len(done)] - c * M)) // 8 * 8
                        piece()
                        val = _tie(val, row, done[-1] & zvec)
                    return val

                for i in range(P):
                    rows = pl.ds(pl.multiple_of((bp0 + i) * Sq, 16), Sq)

                    def pv(j, pb, last):
                        o = jnp.dot(pb, vbuf[sm1, i, j * KC:(j + 1) * KC, :], preferred_element_type=f32)
                        if j > 0:
                            op = ou_all[otile, rows, :]
                            o = o + jnp.concatenate([jnp.concatenate(
                                [op[r * TPQ + c] for c in range(TPQ)], axis=1) for r in range(rep)], axis=0)
                        vals = [o[:, c * 128:(c + 1) * 128] for c in range(TPQ)]
                        vals[0] = paced(vals[0])
                        if last:
                            res = dict(zip(pieces, done, strict=True))
                            step = M // 8 // NGRP * 8
                            per = len(RGS) // NGRP
                            for g in range(NGRP):
                                vals[0] = _tie(vals[0], g * step, qs[z2, 0, 0:8, :] & zvec)
                                grp = RGS[g * per:(g + 1) * per]
                                pi, r0 = grp[0]
                                assert grp[-1][0] == pi
                                qs[pi + z1, :, r0 // 2:r0 // 2 + 8 * per, :] = jnp.stack(
                                    [jnp.concatenate([res[rg_ + (ct,)] for rg_ in grp], axis=0)
                                     for ct in range(TPH)])
                        ou_all[otile, rows, :] = jnp.stack(
                            [vals[c][r * Sq:(r + 1) * Sq] for r in range(rep) for c in range(TPQ)])

                    for j in range(NC):
                        ks = slice(j * KC, (j + 1) * KC)
                        last = i == P - 1 and j == NC - 1
                        pb, l = probs(i, ks)
                        l = l.reshape(rep, Sq, 128)
                        if j > 0:
                            l = l + l_all[ltile, rows, :]
                        l_all[ltile, rows, :] = l
                        if not last:
                            pv(j, pb, False)
                        if i == 0 and j == 0:
                            @pl.when(t + 1 < NS)
                            def _():
                                kcopy(t + 1, sm1).start()

                            vcopy(t, s0).start()

                            @pl.when(t == NS - 2)
                            def _():
                                for cc in wocs:
                                    cc.start()
                        s = lax.dot_general(load_q(qs, i), kbuf[s0, i, ks, :], NT, preferred_element_type=f32)
                        s_scr[i, :, ks] = jnp.concatenate([paced(s[:, 0:128]), s[:, 128:]], axis=1)
                        mrun = colmax(s, mr_scr[z1] if j > 0 else None)
                        if j < NC - 1:
                            mr_scr[z1] = mrun
                        else:
                            m_scr[i] = rowmax(mrun)
                        if last:
                            pv(j, pb, True)
                return (s0, sm1)

            fin = lax.fori_loop(1, NS, body, (jnp.int32(0), jnp.int32(1)))
            zsm[0] = fin[0] * fin[1]

        def back(ou7, l7, accT, acc_n, on0):
            zero = zsm[0]

            def rows_of(big, small, idx_big, idx_small, r0, r1):
                parts = []
                if r0 < HR:
                    parts.append(big[idx_big, r0:min(r1, HR), :])
                if r1 > HR:
                    parts.append(small[idx_small, max(r0, HR) - HR:r1 - HR, :])
                return parts[0] if len(parts) == 1 else jnp.concatenate(parts, axis=0)

            def denom7(n):
                r0, r1 = n * 128, (n + 1) * 128
                return [jnp.broadcast_to(
                    jnp.sum(rows_of(l_all, l7, (Hkv - 1) * rep + r, r, r0, r1), axis=-1, keepdims=True), (128, 128))
                    for r in range(rep)]

            def normed7(n, ls):
                r0, r1 = n * 128, (n + 1) * 128
                tiles = []
                for r in range(rep):
                    rc = _recip(ls[r])
                    for cc in range(TPQ):
                        k = r * TPQ + cc
                        tiles.append(rows_of(ou_all, ou7, (Hkv - 1) * TPH + k, k, r0, r1) * rc)
                return jnp.concatenate(tiles, axis=1).astype(bf16)

            vlast = (NS - 1) % 2
            vcopy(NS - 1, vlast).wait()
            for cc in wocs:
                cc.wait()

            def cbody(ii, c):
                for u in range(CU):
                    i = ii * CU + u
                    rows = pl.ds(pl.multiple_of(i * Sq, 16), Sq)
                    o = None
                    l = None
                    for k0 in range(0, Sk, KCE):
                        pb, lj = probs(i, slice(k0, k0 + KCE))
                        l = lj if l is None else l + lj
                        if k0 + KCE == Sk:
                            l7[:, rows, :] = l.reshape(rep, Sq, 128)
                        oj = jnp.dot(pb, vbuf[vlast, i, k0:k0 + KCE, :], preferred_element_type=f32)
                        o = oj if o is None else oj + o
                    ou7[:, rows, :] = jnp.stack(
                        [o[r * Sq:(r + 1) * Sq, cc * 128:(cc + 1) * 128] for r in range(rep) for cc in range(TPQ)])
                tiles = []
                for k2 in range(CU * G // TPQ):
                    kq = ii * (CU * G // TPQ) + k2
                    rc = _recip(jnp.sum(l_all[kq], axis=-1, keepdims=True))
                    for cc in range(TPQ):
                        tiles.append(ou_all[kq * TPQ + cc] * rc)
                on = jnp.concatenate(tiles, axis=1).astype(bf16)
                w = jnp.concatenate([wor_v[ii * CU + u] for u in range(CU)], axis=1)
                y = lax.dot_general(w, on, NT, preferred_element_type=f32) + jnp.where(ii > 0, accT[...], 0.0)
                for n in range(NPRE):
                    on0[n] = pltpu.bitcast(normed7(n, denom7(n)), i32)
                accT[...] = y
                return c

            lax.fori_loop(0, P // CU, cbody, 0)

            dens = {n: denom7(n) for n in range(NPRE, NO)}
            dep = None
            for n in dens:
                for l in dens[n]:
                    for u in range(16):
                        b = _bits(l[u * 8:u * 8 + 8])
                        dep = b if dep is None else dep | b
            dep = dep & jnp.full((8, 128), zero, i32)

            def after_sums(v):
                for row in range(0, D, 128):
                    v = _tie(v, row, dep)
                return v

            acc_n[...] = after_sums(accT[:, R - 128:R]).T
            ocs = []
            res = {}
            for n in range(NO + LAG):
                if n >= LAG:
                    r0 = (n - LAG) * 128
                    out_v[pl.ds(pl.multiple_of(r0 + zero, 128), 128), :] = res.pop(n - LAG)
                    oc = pltpu.make_async_copy(
                        out_v.at[pl.ds(r0, 128)], out_hbm.at[pl.ds(r0, 128)], osem.at[n - LAG])
                    oc.start()
                    ocs.append(oc)
                if n >= NO:
                    continue
                r0, r1 = n * 128, (n + 1) * 128
                on = normed7(n, dens[n]) if n >= NPRE else pltpu.bitcast(on0[n], bf16)
                if n >= LAG:
                    rows = pl.ds(pl.multiple_of(r0 + zero, 128), 128)
                    out_v[rows, 0:128] = on[:, 0:128]
                    on = jnp.concatenate([out_v[rows, 0:128], on[:, 128:]], axis=1)
                if n == NO - 1:
                    res[n] = (lax.dot_general(on, wo7_v[...], NT, preferred_element_type=f32)
                              + acc_n[...]).astype(bf16)
                else:
                    y = lax.dot_general(wo7_v[...], on, NT, preferred_element_type=f32) + accT[:, r0:r1]
                    res[n] = (after_sums(y) if n < 2 else y).astype(bf16).T
            for oc in ocs:
                oc.wait()

        def stage(u, c):
            @pl.when(u == 0)
            def _():
                pl.run_scoped(
                    front,
                    pltpu.VMEM((2, P, Sk, Dh), bf16),
                    pltpu.VMEM((P, TPH, Sq // 2, 128), i32),
                    pltpu.VMEM((P, TPH, Sq // 2, 128), i32),
                    pltpu.VMEM((NTL - TPH, R // 8, 8, 128), f32),
                    pltpu.VMEM((2, M, 128), f32),
                    pltpu.VMEM((KR, R // 8 + 1, 8, 128), f32),
                    pltpu.VMEM((NTL - TPH, KR, 8, 128), f32),
                )

            @pl.when(u == 1)
            def _():
                pl.run_scoped(
                    back,
                    pltpu.VMEM((TPH, HR, 128), f32),
                    pltpu.VMEM((rep, HR, 128), f32),
                    pltpu.VMEM((D, R), f32),
                    pltpu.VMEM((128, D), f32),
                    pltpu.VMEM((NPRE, 64, W), i32),
                )
            return c

        lax.fori_loop(0, 2, stage, 0)

    out = pl.pallas_call(
        kernel,
        in_specs=[pl.BlockSpec(memory_space=pl.ANY)] * 5,
        out_specs=pl.BlockSpec(memory_space=pl.ANY),
        out_shape=jax.ShapeDtypeStruct((R, D), x.dtype),
        scratch_shapes=[
            pltpu.VMEM((R, D), bf16),
            pltpu.VMEM((D, W), bf16),
            pltpu.VMEM((P, D, G * 128), bf16),
            pltpu.VMEM((2, P, Sk, Dh), bf16),
            pltpu.VMEM((NTL, R, 128), f32),
            pltpu.VMEM((Hq, R, 128), f32),
            pltpu.VMEM((P, M, Sk), f32),
            pltpu.VMEM((P, M, 128), f32),
            pltpu.SMEM((1,), i32),
            pltpu.SemaphoreType.DMA((2,)),
            pltpu.SemaphoreType.DMA((2,)),
            pltpu.SemaphoreType.DMA((P,)),
            pltpu.SemaphoreType.DMA((P,)),
            pltpu.SemaphoreType.DMA((4,)),
            pltpu.SemaphoreType.DMA((NO,)),
        ],
        compiler_params=pltpu.CompilerParams(
            vmem_limit_bytes=127 * 1024 * 1024,
            disable_bounds_checks=True,
            disable_semaphore_checks=True,
        ),
    )(x.reshape(R, D), k_cache, v_cache, wq, wo.T)
    return out.reshape(B, Sq, D)
```

```python
import functools

import jax
import jax.numpy as jnp
from jax import lax
import jax.experimental.pallas as pl
import jax.experimental.pallas.tpu as pltpu

LOG2E = 1.4426950408889634
f32, bf16, i32 = jnp.float32, jnp.bfloat16, jnp.int32
NT = (((1,), (1,)), ((), ()))


def _bits(v):
    return lax.bitcast_convert_type(v, i32)


def _flt(v):
    return lax.bitcast_convert_type(v, f32)


def _recip(l):
    r = pl.reciprocal(l, approx=True)
    return r * (2.0 - l * r)


def _tie(val, row, dep):
    parts = [val[:row]] if row else []
    parts.append(_flt(_bits(val[row:row + 8]) | dep))
    if row + 8 < val.shape[0]:
        parts.append(val[row + 8:])
    return jnp.concatenate(parts, axis=0)


P = 4
KC = 256
KCE = 512
X1, X2, C1 = 256, 432, 2
T0ROWS = 192
AROWS0 = 8
AROWS = 4
CU = 2
LAG = 2
NPRE = 4
GS = 8
PRE = 8
LEAD = 42
DELTA = 125.32
NGRP = 12


@jax.jit
def pallas_standalone__gqa_block_cached__near_ridge_kernel(
    x: jax.Array,
    k_cache: jax.Array,
    v_cache: jax.Array,
    wq: jax.Array,
    wo: jax.Array,
):
    B, Sq, D = x.shape
    _, Hkv, Sk, Dh = k_cache.shape
    Hq = wq.shape[1] // Dh
    rep = Hq // Hkv
    M = rep * Sq
    W = rep * Dh
    R = B * Sq
    TPH = W // 128
    TPQ = Dh // 128
    NTL = Hq * Dh // 128
    G = (NTL - 2 * TPH) // (P - 1)
    HG = G // TPH
    NWB = HG * (P - 1)
    CG = (NTL - TPH) // (P // CU)
    DM = (D // 128) * 128
    KR = D - DM
    NS = B * Hkv // P
    HR = P * Sq
    NO = R // 128
    TR = (R - T0ROWS) // (P - 1)
    assert G * (P - 1) == NTL - 2 * TPH and B == 2 * P and R % 128 == 0 and Sq % 16 == 0 and TR % 16 == 0
    assert TR * (P - 1) + T0ROWS == R and P // CU == 2 and CG == (NWB // 2) * TPH + TPH // 2
    assert KR % GS == 0 and PRE % GS == 0 and CG % TPQ == 0
    scale = Dh ** -0.5 * LOG2E

    def kernel(x_hbm, k_hbm, v_hbm, wq_hbm, wo_hbm, out_hbm,
               x_v, wq0_v, wqx_v, wqr_v, vbuf, ou_all, l_all, s_scr, m_scr, zsm,
               ksem, vsem, k0sem, wqsem, wsem, osem):
        wo7_v, out_v = wq0_v, x_v

        def blk(t):
            if isinstance(t, int):
                return t // 2, (t % 2) * P
            return lax.shift_right_logical(t, 1), (t & 1) * P

        def vcopy(t, slot):
            h, b0 = blk(t)
            return pltpu.make_async_copy(v_hbm.at[pl.ds(b0, P), h], vbuf.at[slot], vsem.at[slot])

        wocs = []
        for ii in range(2):
            for u in range(NWB // 2):
                wocs.append(pltpu.make_async_copy(
                    wo_hbm.at[:, pl.ds(ii * CG * 128 + u * W, W)], wqr_v.at[ii * (NWB // 2) + u], wsem.at[3]))
            wocs.append(pltpu.make_async_copy(
                wo_hbm.at[:, pl.ds((ii + 1) * CG * 128 - W // 2, W // 2)], wqx_v.at[ii], wsem.at[3]))
        wocs.append(pltpu.make_async_copy(wo_hbm.at[:, pl.ds(2 * CG * 128, W)], wo7_v, wsem.at[3]))

        def xcopy(r0, r1, sem):
            return pltpu.make_async_copy(x_hbm.at[pl.ds(r0, r1 - r0)], x_v.at[pl.ds(r0, r1 - r0)], sem)

        def w0copy(t0, t1, sem):
            cols = pl.ds(t0 * 128, (t1 - t0) * 128)
            return pltpu.make_async_copy(wq_hbm.at[:, cols], wq0_v.at[:, cols], sem)

        firsts = [[w0copy(0, C1, wsem.at[0]), xcopy(0, X1, wsem.at[0])],
                  [w0copy(C1, TPH, wsem.at[1]), xcopy(X1, X2, wsem.at[1])],
                  [xcopy(X2, R, wsem.at[2])]]
        for grp in firsts:
            for cc in grp:
                cc.start()

        def probs(i, ks):
            nt = (ks.stop - ks.start) // 128
            p = jnp.exp2(s_scr[i, :, ks] - jnp.concatenate([m_scr[i]] * nt, axis=1))
            l = p[:, 0:128]
            for c in range(1, nt):
                l = l + p[:, c * 128:(c + 1) * 128]
            return p.astype(bf16), l

        def front(zero0, kbuf, q0, qs, qa, mr_scr, xB, wB):
            def kcopy(t, slot):
                h, b0 = blk(t)
                return pltpu.make_async_copy(k_hbm.at[pl.ds(b0, P), h], kbuf.at[slot], ksem.at[slot])

            def k0copy(i):
                return pltpu.make_async_copy(k_hbm.at[i, 0], kbuf.at[0, i], k0sem.at[i])

            def wqrc(i):
                if isinstance(i, int) and i == 0:
                    return [pltpu.make_async_copy(wq_hbm.at[:, pl.ds(W + u * W // 2, W // 2)], wqx_v.at[u],
                                                  wqsem.at[0]) for u in range(2)]
                return [pltpu.make_async_copy(wq_hbm.at[:, pl.ds((2 + (i - 1) * HG + u) * W, W)],
                                              wqr_v.at[(i - 1) * HG + u], wqsem.at[i]) for u in range(HG)]

            def qproj0(r0, r1, t0, t1):
                q = jnp.dot(x_v[r0:r1, :], wq0_v[:, t0 * 128:t1 * 128], preferred_element_type=f32)
                q = pltpu.bitcast((q * scale).astype(bf16), i32)
                for b in range(B):
                    a0, a1 = max(r0, b * Sq), min(r1, (b + 1) * Sq)
                    if a0 >= a1:
                        continue
                    qb = q[(a0 - r0) // 2:(a1 - r0) // 2]
                    val = jnp.stack([qb[:, k * 128:(k + 1) * 128] for k in range(t1 - t0)])
                    (q0 if b < P else qs)[b % P, t0:t1, (a0 - b * Sq) // 2:(a1 - b * Sq) // 2, :] = val

            for cc in firsts[0]:
                cc.wait()
            for cc in wqrc(0):
                cc.start()
            k0copy(0).start()
            qproj0(0, X1, 0, C1)
            for cc in firsts[1]:
                cc.wait()
            qproj0(X1, X2, 0, C1)
            qproj0(0, X2, C1, TPH)
            for cc in firsts[2]:
                cc.wait()
            k0copy(1).start()
            for cc in wqrc(1):
                cc.start()
            qproj0(X2, R, 0, TPH)

            def load_q(ref, i):
                q = ref[i]
                return pltpu.bitcast(jnp.concatenate(
                    [jnp.concatenate([q[r * TPQ + c] for c in range(TPQ)], axis=1) for r in range(rep)],
                    axis=0), bf16)

            def colmax(s, mrun):
                for c in range(s.shape[1] // 128):
                    sc = s[:, c * 128:(c + 1) * 128]
                    mrun = sc if mrun is None else jnp.maximum(mrun, sc)
                return mrun

            def rowmax(mrun):
                return jnp.broadcast_to(jnp.max(mrun, axis=-1, keepdims=True), (M, 128))

            def astep(i, z, getw, ng, tile0, trow0, tr, nrows):
                k0copy(i).wait()
                for cc in wqrc(i):
                    cc.wait()
                zv = jnp.full((8, 128), z, i32)
                rg = R // nrows

                def start_when(cond, copies):
                    def go():
                        for cc in copies():
                            cc.start()

                    if not isinstance(cond, bool):
                        pl.when(cond)(go)
                    elif cond:
                        go()

                start_when(i + 2 < P, lambda: wqrc(i + 2))
                start_when(i + 2 < P, lambda: [k0copy(i + 2)])
                start_when(i == 1, lambda: [kcopy(1, 1)])
                start_when(i == 2, lambda: [vcopy(0, 0)])

                def qpart(g):
                    q = jnp.dot(x_v[g * rg:(g + 1) * rg, 0:DM], getw(0, DM), preferred_element_type=f32)
                    q = q * scale
                    qa[pl.ds(tile0, ng), g * rg // 8:(g + 1) * rg // 8] = jnp.stack(
                        [q[:, k * 128:(k + 1) * 128].reshape(rg // 8, 8, 128) for k in range(ng)])
                    return q

                qp = qpart(0)
                mrun = None
                for k0 in range(0, Sk, KCE):
                    s = lax.dot_general(load_q(q0, i), kbuf[0, i, k0:k0 + KCE, :], NT,
                                        preferred_element_type=f32)
                    s_scr[i, :, k0:k0 + KCE] = s
                    mrun = colmax(s, mrun)
                mx = rowmax(mrun)
                m_scr[i] = mx
                for g in range(1, nrows):
                    qpart(g)

                dep = _bits(mx[M - 8:M])
                for u in range(2, M // 8 + 1):
                    dep = dep | _bits(mx[M - 8 * u:M - 8 * u + 8])
                dep = jnp.concatenate([(dep & zv)[:, 0:KR]] * (tr // 16), axis=0)
                rs = trow0 if isinstance(trow0, int) else pl.multiple_of(trow0, 16)
                xr = x_v[pl.ds(rs, tr), DM:D]
                xr = pltpu.bitcast(pltpu.bitcast(xr, i32) | dep, bf16).astype(f32)
                xB[:, pl.ds(trow0 // 8, tr // 8)] = jnp.stack(
                    [jnp.broadcast_to(xr[:, kk:kk + 1], (tr, 128)).reshape(tr // 8, 8, 128) for kk in range(KR)])
                wr = getw(DM, D).astype(f32) * scale
                nrg = rg // 8
                wrows = []
                for kk in range(KR):
                    n = kk * (nrg * ng) // KR
                    dep = _bits(qp[(n % nrg) * 8:(n % nrg) * 8 + 8, (n // nrg) * 128:(n // nrg + 1) * 128]) & zv
                    wrow = jnp.broadcast_to(wr[kk:kk + 1, :], (8, ng * 128))
                    wrows.append(_flt(_bits(wrow) | jnp.concatenate([dep] * ng, axis=1)))
                wall = jnp.stack(wrows)
                wB[pl.ds(tile0, ng)] = jnp.stack([wall[:, :, k * 128:(k + 1) * 128] for k in range(ng)])

            astep(0, zero0, lambda a, b: jnp.concatenate([wqx_v[u, a:b, :] for u in range(2)], axis=1),
                  TPH, 0, 0, T0ROWS, AROWS0)

            def abody(i, zc):
                astep(i, zc[0] * zc[1],
                      lambda a, b: jnp.concatenate([wqr_v[(i - 1) * HG + u, a:b, :] for u in range(HG)], axis=1),
                      G, TPH + (i - 1) * G, T0ROWS + (i - 1) * TR, TR, AROWS)
                return (zc[1], zc[0])

            lax.fori_loop(1, P, abody, (jnp.int32(0), jnp.int32(1)))

            NC = Sk // KC
            RGS = [(i, r0) for i in range(P) for r0 in range(0, Sq, 16)]
            pieces = [RGS[n % len(RGS)] + ((n + n // len(RGS)) % TPH,) for n in range(len(RGS) * TPH)]
            assert len(set(pieces)) == len(pieces)
            due = [2 * NC * P * M - LEAD - (len(pieces) - 1 - n) * DELTA for n in range(len(pieces))]

            def body(t, slots):
                sm1, s0 = slots
                kcopy(t, s0).wait()
                vcopy(t - 1, sm1).wait()
                hp, bp0 = blk(t - 1)
                hn, bn0 = blk(jnp.minimum(t + 1, NS - 1))
                z1 = sm1 * s0
                z2 = sm1 + s0 - 1
                zvec = jnp.full((8, 128), z1, i32)
                wt = [(hn - 1) * TPH + ct for ct in range(TPH)]
                otile = pl.ds(hp * TPH, TPH)
                ltile = pl.ds(hp * rep, rep)
                rg0 = bn0 * (Sq // 8)
                done = []
                nmm = [0]

                def piece():
                    i, r0, ct = pieces[len(done)]
                    rows = pl.ds(rg0 + (i * Sq + r0) // 8, 2)
                    acc = qa[wt[ct], rows][None]
                    for k0 in range(0, KR, GS):
                        xg = xB[k0:k0 + GS, rows]
                        wg = wB[wt[ct], k0:k0 + GS][:, None]
                        if k0 == PRE and done:
                            acc = _flt(_bits(acc) | (done[-1] & zvec)[None, None])
                        acc = jnp.sum(jnp.concatenate([acc, xg * wg], axis=0), axis=0, keepdims=True)
                    done.append(pltpu.bitcast(acc.reshape(16, 128).astype(bf16), i32))

                def paced(val):
                    c = nmm[0]
                    nmm[0] += 1
                    while len(done) < len(pieces) and due[len(done)] < (c + 1) * M:
                        row = max(0, int(due[len(done)] - c * M)) // 8 * 8
                        piece()
                        val = _tie(val, row, done[-1] & zvec)
                    return val

                for i in range(P):
                    rows = pl.ds(pl.multiple_of((bp0 + i) * Sq, 16), Sq)

                    def pv(j, pb, last):
                        o = jnp.dot(pb, vbuf[sm1, i, j * KC:(j + 1) * KC, :], preferred_element_type=f32)
                        if j > 0:
                            op = ou_all[otile, rows, :]
                            o = o + jnp.concatenate([jnp.concatenate(
                                [op[r * TPQ + c] for c in range(TPQ)], axis=1) for r in range(rep)], axis=0)
                        vals = [o[:, c * 128:(c + 1) * 128] for c in range(TPQ)]
                        vals[0] = paced(vals[0])
                        if last:
                            res = dict(zip(pieces, done, strict=True))
                            step = M // 8 // NGRP * 8
                            per = len(RGS) // NGRP
                            for g in range(NGRP):
                                vals[0] = _tie(vals[0], g * step, qs[z2, 0, 0:8, :] & zvec)
                                grp = RGS[g * per:(g + 1) * per]
                                pi, r0 = grp[0]
                                assert grp[-1][0] == pi
                                qs[pi + z1, :, r0 // 2:r0 // 2 + 8 * per, :] = jnp.stack(
                                    [jnp.concatenate([res[rg_ + (ct,)] for rg_ in grp], axis=0)
                                     for ct in range(TPH)])
                        ou_all[otile, rows, :] = jnp.stack(
                            [vals[c][r * Sq:(r + 1) * Sq] for r in range(rep) for c in range(TPQ)])

                    for j in range(NC):
                        ks = slice(j * KC, (j + 1) * KC)
                        last = i == P - 1 and j == NC - 1
                        pb, l = probs(i, ks)
                        l = l.reshape(rep, Sq, 128)
                        if j > 0:
                            l = l + l_all[ltile, rows, :]
                        l_all[ltile, rows, :] = l
                        if not last:
                            pv(j, pb, False)
                        if i == 0 and j == 0:
                            @pl.when(t + 1 < NS)
                            def _():
                                kcopy(t + 1, sm1).start()

                            vcopy(t, s0).start()

                            @pl.when(t == NS - 2)
                            def _():
                                for cc in wocs:
                                    cc.start()
                        s = lax.dot_general(load_q(qs, i), kbuf[s0, i, ks, :], NT, preferred_element_type=f32)
                        s_scr[i, :, ks] = jnp.concatenate([paced(s[:, 0:128]), s[:, 128:]], axis=1)
                        mrun = colmax(s, mr_scr[z1] if j > 0 else None)
                        if j < NC - 1:
                            mr_scr[z1] = mrun
                        else:
                            m_scr[i] = rowmax(mrun)
                        if last:
                            pv(j, pb, True)
                return (s0, sm1)

            fin = lax.fori_loop(1, NS, body, (jnp.int32(0), jnp.int32(1)))
            zsm[0] = fin[0] * fin[1]

        def back(ou7, l7, accT, acc_n, on0):
            zero = zsm[0]

            def rows_of(big, small, idx_big, idx_small, r0, r1):
                parts = []
                if r0 < HR:
                    parts.append(big[idx_big, r0:min(r1, HR), :])
                if r1 > HR:
                    parts.append(small[idx_small, max(r0, HR) - HR:r1 - HR, :])
                return parts[0] if len(parts) == 1 else jnp.concatenate(parts, axis=0)

            def denom7(n):
                r0, r1 = n * 128, (n + 1) * 128
                return [jnp.broadcast_to(
                    jnp.sum(rows_of(l_all, l7, (Hkv - 1) * rep + r, r, r0, r1), axis=-1, keepdims=True), (128, 128))
                    for r in range(rep)]

            def normed7(n, ls):
                r0, r1 = n * 128, (n + 1) * 128
                tiles = []
                for r in range(rep):
                    rc = _recip(ls[r])
                    for cc in range(TPQ):
                        k = r * TPQ + cc
                        tiles.append(rows_of(ou_all, ou7, (Hkv - 1) * TPH + k, k, r0, r1) * rc)
                return jnp.concatenate(tiles, axis=1).astype(bf16)

            vlast = (NS - 1) % 2
            vcopy(NS - 1, vlast).wait()
            for cc in wocs:
                cc.wait()

            def cbody(ii, c):
                for u in range(CU):
                    i = ii * CU + u
                    rows = pl.ds(pl.multiple_of(i * Sq, 16), Sq)
                    o = None
                    l = None
                    for k0 in range(0, Sk, KCE):
                        pb, lj = probs(i, slice(k0, k0 + KCE))
                        l = lj if l is None else l + lj
                        if k0 + KCE == Sk:
                            l7[:, rows, :] = l.reshape(rep, Sq, 128)
                        oj = jnp.dot(pb, vbuf[vlast, i, k0:k0 + KCE, :], preferred_element_type=f32)
                        o = oj if o is None else oj + o
                    ou7[:, rows, :] = jnp.stack(
                        [o[r * Sq:(r + 1) * Sq, cc * 128:(cc + 1) * 128] for r in range(rep) for cc in range(TPQ)])
                tiles = []
                for k2 in range(CG // TPQ):
                    kq = ii * (CG // TPQ) + k2
                    rc = _recip(jnp.sum(l_all[kq], axis=-1, keepdims=True))
                    for cc in range(TPQ):
                        tiles.append(ou_all[kq * TPQ + cc] * rc)
                on = jnp.concatenate(tiles, axis=1).astype(bf16)
                w = jnp.concatenate([wqr_v[ii * (NWB // 2) + u] for u in range(NWB // 2)] + [wqx_v[ii]], axis=1)
                y = lax.dot_general(w, on, NT, preferred_element_type=f32) + jnp.where(ii > 0, accT[...], 0.0)
                for n in range(NPRE):
                    on0[n] = pltpu.bitcast(normed7(n, denom7(n)), i32)
                accT[...] = y
                return c

            lax.fori_loop(0, P // CU, cbody, 0)

            dens = {n: denom7(n) for n in range(NPRE, NO)}
            dep = None
            for n in dens:
                for l in dens[n]:
                    for u in range(16):
                        b = _bits(l[u * 8:u * 8 + 8])
                        dep = b if dep is None else dep | b
            dep = dep & jnp.full((8, 128), zero, i32)

            def after_sums(v):
                for row in range(0, D, 128):
                    v = _tie(v, row, dep)
                return v

            acc_n[...] = after_sums(accT[:, R - 128:R]).T
            ocs = []
            res = {}
            for n in range(NO + LAG):
                if n >= LAG:
                    r0 = (n - LAG) * 128
                    out_v[pl.ds(pl.multiple_of(r0 + zero, 128), 128), :] = res.pop(n - LAG)
                    oc = pltpu.make_async_copy(
                        out_v.at[pl.ds(r0, 128)], out_hbm.at[pl.ds(r0, 128)], osem.at[n - LAG])
                    oc.start()
                    ocs.append(oc)
                if n >= NO:
                    continue
                r0, r1 = n * 128, (n + 1) * 128
                on = normed7(n, dens[n]) if n >= NPRE else pltpu.bitcast(on0[n], bf16)
                if n >= LAG:
                    rows = pl.ds(pl.multiple_of(r0 + zero, 128), 128)
                    out_v[rows, 0:128] = on[:, 0:128]
                    on = jnp.concatenate([out_v[rows, 0:128], on[:, 128:]], axis=1)
                if n == NO - 1:
                    res[n] = (lax.dot_general(on, wo7_v[...], NT, preferred_element_type=f32)
                              + acc_n[...]).astype(bf16)
                else:
                    y = lax.dot_general(wo7_v[...], on, NT, preferred_element_type=f32) + accT[:, r0:r1]
                    res[n] = (after_sums(y) if n < 2 else y).astype(bf16).T
            for oc in ocs:
                oc.wait()

        def stage(u, c):
            @pl.when(u == 0)
            def _():
                pl.run_scoped(
                    functools.partial(front, u),
                    pltpu.VMEM((2, P, Sk, Dh), bf16),
                    pltpu.VMEM((P, TPH, Sq // 2, 128), i32),
                    pltpu.VMEM((P, TPH, Sq // 2, 128), i32),
                    pltpu.VMEM((NTL - TPH, R // 8, 8, 128), f32),
                    pltpu.VMEM((2, M, 128), f32),
                    pltpu.VMEM((KR, R // 8 + 1, 8, 128), f32),
                    pltpu.VMEM((NTL - TPH, KR, 8, 128), f32),
                )

            @pl.when(u == 1)
            def _():
                pl.run_scoped(
                    back,
                    pltpu.VMEM((TPH, HR, 128), f32),
                    pltpu.VMEM((rep, HR, 128), f32),
                    pltpu.VMEM((D, R), f32),
                    pltpu.VMEM((128, D), f32),
                    pltpu.VMEM((NPRE, 64, W), i32),
                )
            return c

        lax.fori_loop(0, 2, stage, 0)

    out = pl.pallas_call(
        kernel,
        in_specs=[pl.BlockSpec(memory_space=pl.ANY)] * 5,
        out_specs=pl.BlockSpec(memory_space=pl.ANY),
        out_shape=jax.ShapeDtypeStruct((R, D), x.dtype),
        scratch_shapes=[
            pltpu.VMEM((R, D), bf16),
            pltpu.VMEM((D, W), bf16),
            pltpu.VMEM((2, D, W // 2), bf16),
            pltpu.VMEM((NWB, D, W), bf16),
            pltpu.VMEM((2, P, Sk, Dh), bf16),
            pltpu.VMEM((NTL, R, 128), f32),
            pltpu.VMEM((Hq, R, 128), f32),
            pltpu.VMEM((P, M, Sk), f32),
            pltpu.VMEM((P, M, 128), f32),
            pltpu.SMEM((1,), i32),
            pltpu.SemaphoreType.DMA((2,)),
            pltpu.SemaphoreType.DMA((2,)),
            pltpu.SemaphoreType.DMA((P,)),
            pltpu.SemaphoreType.DMA((P,)),
            pltpu.SemaphoreType.DMA((4,)),
            pltpu.SemaphoreType.DMA((NO,)),
        ],
        compiler_params=pltpu.CompilerParams(
            vmem_limit_bytes=127 * 1024 * 1024,
            disable_bounds_checks=True,
            disable_semaphore_checks=True,
        ),
    )(x.reshape(R, D), k_cache, v_cache, wq, wo.T)
    return out.reshape(B, Sq, D)
```
